```python
import os as _os
_os.environ.setdefault('JAX_PLATFORMS', 'cpu')
import jax
import jax.numpy as jnp

def _softmax(x, axis=-1):
    return jax.nn.softmax(x, axis=axis)

def _gelu(x):
    return jax.nn.gelu(x, approximate=True)

def _silu(x):
    return jax.nn.silu(x)

def _sigmoid(x):
    return jax.nn.sigmoid(x)

def _layernorm(x, axis=-1, eps=1e-05):
    m = jnp.mean(x, axis=axis, keepdims=True)
    v = jnp.var(x, axis=axis, keepdims=True)
    return (x - m) / jnp.sqrt(v + eps)

def _scatter_add(tgt, idx, src, axis=0):
    return tgt.at[idx].add(src)

def _segment_sum(src, seg, n):
    return jax.ops.segment_sum(src, seg, n)

class _Rng:

    def __init__(self, key):
        self._k = key

    def _next(self):
        self._k, sub = jax.random.split(self._k)
        return sub

    def normal(self, shape):
        return jax.random.normal(self._next(), shape, dtype=jnp.bfloat16)

    def randint(self, lo, hi, shape):
        return jax.random.randint(self._next(), shape, lo, hi, dtype=jnp.int32)

    def uniform(self, shape, lo=0.0, hi=1.0):
        return jax.random.uniform(self._next(), shape, jnp.bfloat16, lo, hi)

    def permutation(self, n):
        return jax.random.permutation(self._next(), n)
kernel_name = 'gated_mix__mha_block__memory_aug_recurrent_mem_tr__prompt'

def setup_inputs():
    _rng = _Rng(jax.random.key(int.from_bytes(__import__("os").urandom(4), "little")))
    _w = lambda a: (lambda t: t.astype(jnp.bfloat16) if jnp.issubdtype(t.dtype, jnp.floating) else t)(jnp.asarray(a))

    def _A_setup():
        B, S, D, H = (1, 2048, 512, 32)
        return {'x': _w((lambda *s: _rng.normal(s) * 0.05)(B, S, D)), 'wqkv': _w((lambda *s: _rng.normal(s) * 0.8)(D, 3 * D)), 'wo': _w((lambda *s: _rng.normal(s) * 0.05)(D, D))}
    _A_in = _A_setup()

    def _B_setup():
        B, S, Dm = (1, 2048, 512)
        H, Dh = (32, 128)
        M, seg = (8, 32)
        seg = min(seg, S)
        S = S // seg * seg
        return {'x': _w((lambda *s: _rng.normal(s) * 0.05)(B, S, Dm)), 'mem0': _w((lambda *s: _rng.normal(s) * 0.8)(B, M, Dm)), 'Wq': _w((lambda *s: _rng.normal(s) * 1.6)(Dm, H, Dh) * Dm ** (-0.5)), 'Wk': _w((lambda *s: _rng.normal(s) * 1.6)(Dm, H, Dh) * Dm ** (-0.5)), 'Wv': _w((lambda *s: _rng.normal(s) * 0.8)(Dm, H, Dh) * Dm ** (-0.5)), 'Wo': _w((lambda *s: _rng.normal(s) * 0.8)(H, Dh, Dm) * (H * Dh) ** (-0.5)), 'seg_len': seg}
    _B_in = _B_setup()
    return {'A_x': _A_in['x'], 'A_wqkv': _A_in['wqkv'], 'A_wo': _A_in['wo'], 'B_x': _B_in['x'], 'B_mem0': _B_in['mem0'], 'B_Wq': _B_in['Wq'], 'B_Wk': _B_in['Wk'], 'B_Wv': _B_in['Wv'], 'B_Wo': _B_in['Wo'], 'B_seg_len': _B_in['seg_len'], 'gate_w': _w((lambda *s: _rng.normal(s) * 0.05)(512) * 16.0)}

def reference(A_x, A_wqkv, A_wo, B_x, B_mem0, B_Wq, B_Wk, B_Wv, B_Wo, B_seg_len, gate_w):

    def _A_ref(x, wqkv, wo):
        B, S, D = x.shape
        H = 32
        Dh = D // H
        qkv = (lambda x, *d: x.transpose(*d))((x @ wqkv).reshape(B, S, 3, H, Dh), 2, 0, 3, 1, 4)
        q, k, v = (qkv[0], qkv[1], qkv[2])
        scores = jnp.einsum('bhqd,bhkd->bhqk', q, k) * Dh ** (-0.5)
        p = _softmax(scores, axis=-1)
        o = jnp.einsum('bhqk,bhkd->bhqd', p, v)
        return (lambda x, *d: x.transpose(*d))(o, 0, 2, 1, 3).reshape(B, S, D) @ wo

    def _B_ref(x, mem0, Wq, Wk, Wv, Wo, seg_len):
        B, S, Dm = x.shape
        H, Dh = (Wq.shape[1], Wq.shape[2])
        M = mem0.shape[1]
        scale = Dh ** (-0.5)
        n_seg = S // seg_len
        L = M + seg_len
        idx = jnp.arange(L)
        mask = (idx[:, None] < M) | (idx[:, None] >= idx[None, :])
        mem = mem0
        outs = []
        for s in range(n_seg):
            xs = x[:, s * seg_len:(s + 1) * seg_len, :].copy()
            h = jnp.concatenate([mem, xs], axis=1)
            q = jnp.einsum('btd,dhe->bhte', h, Wq)
            k = jnp.einsum('btd,dhe->bhte', h, Wk)
            v = jnp.einsum('btd,dhe->bhte', h, Wv)
            scores = jnp.einsum('bhqe,bhke->bhqk', q, k) * scale
            scores = jnp.where(mask[None, None], scores, -1000000000.0)
            p = _softmax(scores, axis=-1)
            o = jnp.einsum('bhqk,bhke->bhqe', p, v)
            o = jnp.einsum('bhte,hed->btd', o, Wo)
            mem = o[:, :M, :].copy()
            outs.append(o[:, M:, :])
        return jnp.concatenate(outs, axis=1)
    x = A_x
    g = _sigmoid((x * gate_w).sum(-1, keepdims=True))
    a = _A_ref(x, A_wqkv, A_wo)
    b = _B_ref(x, B_mem0, B_Wq, B_Wk, B_Wv, B_Wo, B_seg_len)
    return g * a + (1 - g) * b
```

```python
import functools

import jax
import jax.numpy as jnp
import jax.experimental.pallas as pl
import jax.experimental.pallas.tpu as pltpu

LOG2E = 1.4426950408889634
F32 = jnp.float32
BF16 = jnp.bfloat16
NN = (((1,), (0,)), ((), ()))
NT = (((1,), (1,)), ((), ()))
TN = (((0,), (0,)), ((), ()))
TT = (((0,), (1,)), ((), ()))


def _dot(a, b, dims=NN):
    return jax.lax.dot_general(a, b, dims, preferred_element_type=F32)


def _make_kernel(S, D, HA, HB, DHB, M, SEG):
    DHA = D // HA
    NSEG = S // SEG
    L = M + SEG
    BQ = 512
    BK = 128
    NQ = S // BQ
    NK = S // BK
    NU = HA * NQ
    GH = 128 // DHA
    VR = DHA + 8
    G = 2
    NG = HB // G
    LAGS = (1, 2, 4)

    def kernel(x_ref, wqkv_ref, woa_ref, mem0_ref, gw_ref,
               wq3_hbm, wk3_hbm, wv3_hbm, wob_hbm,
               out_ref,
               ka_ref, qm_ref, vt_ref, sa_ref, sb_ref, ma_ref, mb_ref, ot_ref,
               ga_ref, omg_ref,
               w3_ref, wqkvb_ref, wob_ref, sems):
        copies = [
            pltpu.make_async_copy(wq3_hbm, w3_ref.at[0], sems.at[0]),
            pltpu.make_async_copy(wk3_hbm, w3_ref.at[1], sems.at[1]),
            pltpu.make_async_copy(wv3_hbm, w3_ref.at[2], sems.at[2]),
            pltpu.make_async_copy(wob_hbm, wob_ref, sems.at[3]),
        ]
        for c in copies:
            c.start()

        wq_t = wqkv_ref[:, 0:D].astype(F32).T
        wv_t = wqkv_ref[:, 2 * D:3 * D].astype(F32).T
        gw = jnp.broadcast_to(gw_ref[...], (128, D))
        qscale = (DHA ** -0.5) * LOG2E

        def proj_a(i, _):
            rows = pl.ds(pl.multiple_of(i * BQ, BQ), BQ)
            xb = x_ref[rows, :]
            ka_ref[rows, :] = _dot(xb, wqkv_ref[:, D:2 * D]).astype(BF16)
            qt = (_dot(wq_t, xb, NT) * qscale).astype(BF16)
            vt = _dot(wv_t, xb, NT)
            ones = jnp.ones((VR - DHA, BQ), F32)
            for h in range(HA):
                j = h % GH
                parts = []
                if j > 0:
                    parts.append(jnp.zeros((j * DHA, BQ), BF16))
                parts.append(qt[h * DHA:(h + 1) * DHA])
                if j < GH - 1:
                    parts.append(jnp.zeros(((GH - 1 - j) * DHA, BQ), BF16))
                qm_ref[h * 128:(h + 1) * 128, rows] = jnp.concatenate(parts, axis=0)
                vt_ref[h * VR:h * VR + DHA, rows] = vt[h * DHA:(h + 1) * DHA]
                vt_ref[h * VR + DHA:(h + 1) * VR, rows] = ones
            z = _dot(xb, gw, NT)
            g = jax.nn.sigmoid(z)
            ga_ref[rows, 0:128] = g
            omg_ref[rows, :] = 1.0 - g
            return 0
        jax.lax.fori_loop(0, S // BQ, proj_a, 0)

        def qcols(u):
            return pl.ds(pl.multiple_of((u % NQ) * BQ, BQ), BQ)

        def s_chunk(u, c, buf):
            h = u // NQ
            qm = qm_ref[pl.ds(pl.multiple_of(h * 128, 128), 128), qcols(u)]
            kk = ka_ref[c * BK:(c + 1) * BK, pl.ds(pl.multiple_of((h // GH) * 128, 128), 128)]
            st = _dot(kk, qm)
            buf[c * BK:(c + 1) * BK, :] = st
            return jnp.max(st.reshape(BK // 8, 8, BQ), axis=0)

        def phase(u_s, buf_s, m_s, u_p, buf_p, m_p):
            m = m_p[...]
            hp = u_p // NQ
            r0 = pl.multiple_of(hp * VR, 8)
            ot = jnp.zeros((VR, BQ), F32)
            mx8 = None
            for c in range(NK):
                mc = s_chunk(u_s, c, buf_s)
                mx8 = mc if mx8 is None else jnp.maximum(mx8, mc)
                p = jnp.exp2(buf_p[c * BK:(c + 1) * BK, :] - m)
                ot = ot + _dot(vt_ref[pl.ds(r0, VR), c * BK:(c + 1) * BK], p)
            m_s[...] = jnp.max(mx8, axis=0, keepdims=True)
            ot_ref[pl.ds(pl.multiple_of(hp * DHA, DHA), DHA), qcols(u_p)] = (
                ot[:DHA] / ot[DHA:DHA + 1]).astype(BF16)

        mx8 = None
        for c in range(NK):
            mc = s_chunk(0, c, sa_ref)
            mx8 = mc if mx8 is None else jnp.maximum(mx8, mc)
        ma_ref[...] = jnp.max(mx8, axis=0, keepdims=True)

        def attn_a(i, _):
            u0 = 2 * i
            u1 = u0 + 1
            u2 = jnp.minimum(u0 + 2, NU - 1)
            phase(u1, sb_ref, mb_ref, u0, sa_ref, ma_ref)
            phase(u2, sa_ref, ma_ref, u1, sb_ref, mb_ref)
            return 0
        jax.lax.fori_loop(0, NU // 2, attn_a, 0)

        def proj_o(i, _):
            rows = pl.ds(pl.multiple_of(i * BQ, BQ), BQ)
            a = _dot(ot_ref[:, rows], woa_ref[...], TN)
            a = a.astype(BF16).astype(F32)
            g = ga_ref[rows, 0:128]
            ga_ref[rows, :] = a * jnp.concatenate([g] * (D // 128), axis=1)
            return 0
        jax.lax.fori_loop(0, S // BQ, proj_o, 0)

        for c in copies:
            c.wait()

        def relayout(i, _):
            t = i // (D // 16)
            d0 = pl.multiple_of((i % (D // 16)) * 16, 16)
            blk = w3_ref[t, pl.ds(d0, 16), :, :]
            u = pltpu.bitcast(blk, jnp.uint32)
            tt = jnp.swapaxes(u, 0, 1)
            for hp in range(HB // 2):
                ab = tt[hp]
                lo = pltpu.bitcast(ab << 16, F32).astype(BF16)
                hi = pltpu.bitcast(ab & jnp.uint32(0xFFFF0000), F32).astype(BF16)
                wqkvb_ref[t, pl.ds(d0, 16), (2 * hp) * DHB:(2 * hp + 1) * DHB] = lo
                wqkvb_ref[t, pl.ds(d0, 16), (2 * hp + 1) * DHB:(2 * hp + 2) * DHB] = hi
            return 0
        jax.lax.fori_loop(0, 3 * (D // 16), relayout, 0)

        row = jax.lax.broadcasted_iota(jnp.int32, (L, L), 0)
        col = jax.lax.broadcasted_iota(jnp.int32, (L, L), 1)
        allowed = (row >= SEG) | (col >= SEG) | (col <= row)
        bscale = (DHB ** -0.5) * LOG2E
        lS, lPV, lP = LAGS

        def step(s, mem):
            rows = pl.ds(pl.multiple_of(s * SEG, SEG), SEG)
            h = jnp.concatenate([x_ref[rows, :].astype(F32), mem], axis=0)

            def qkv(g):
                cs = slice(g * G * DHB, (g + 1) * G * DHB)
                return tuple(_dot(h, wqkvb_ref[t, :, cs]) for t in range(3))

            def attn1(q, k, v):
                ps = []
                for j in range(G):
                    hs = slice(j * DHB, (j + 1) * DHB)
                    sc = _dot(q[:, hs], k[:, hs], NT) * bscale
                    sc = jnp.where(allowed, sc, -1e30)
                    m = jnp.max(sc, axis=1, keepdims=True)
                    p = jnp.exp2(sc - m)
                    l = jnp.sum(p, axis=1, keepdims=True)
                    ps.append((p, pl.reciprocal(l, approx=True)))
                return ps

            def attn2(ps, v):
                os_ = []
                for j in range(G):
                    hs = slice(j * DHB, (j + 1) * DHB)
                    p, rl = ps[j]
                    os_.append(_dot(p, v[:, hs]) * rl)
                return jnp.concatenate(os_, axis=1)

            acc = jnp.zeros((L, D), F32)
            QKV, PS, OG = {}, {}, {}
            for g in range(NG + lP):
                if g < NG:
                    QKV[g] = qkv(g)
                if 0 <= g - lS < NG:
                    PS[g - lS] = attn1(*QKV[g - lS])
                if 0 <= g - lPV < NG:
                    OG[g - lPV] = attn2(PS[g - lPV], QKV[g - lPV][2])
                if 0 <= g - lP < NG:
                    gg = g - lP
                    acc = acc + _dot(OG[gg], wob_ref[gg * G * DHB:(gg + 1) * G * DHB, :])
            b = acc[:SEG].astype(BF16).astype(F32)
            omg = omg_ref[rows, :]
            out_ref[rows, :] = (ga_ref[rows, :] + jnp.concatenate([omg] * (D // 128), axis=1) * b).astype(out_ref.dtype)
            return acc[SEG:]

        jax.lax.fori_loop(0, NSEG, step, mem0_ref[...].astype(F32))

    return kernel


@functools.partial(jax.jit, static_argnames=("B_seg_len",))
def pallas_gated_mix__mha_block__memory_aug_recurrent_mem_tr__prompt_kernel(
    A_x, A_wqkv, A_wo, B_x, B_mem0, B_Wq, B_Wk, B_Wv, B_Wo, B_seg_len, gate_w,
):
    del B_x
    Bn, S, D = A_x.shape
    assert Bn == 1
    HA = 32
    _, HB, DHB = B_Wq.shape
    M = B_mem0.shape[1]
    SEG = int(B_seg_len)
    DHA = D // HA
    VR = DHA + 8
    kernel = _make_kernel(S, D, HA, HB, DHB, M, SEG)
    vmem = pl.BlockSpec(memory_space=pltpu.VMEM)
    hbm = pl.BlockSpec(memory_space=pl.ANY)
    out = pl.pallas_call(
        kernel,
        out_shape=jax.ShapeDtypeStruct((S, D), A_x.dtype),
        in_specs=[vmem, vmem, vmem, vmem, vmem, hbm, hbm, hbm, hbm],
        out_specs=vmem,
        scratch_shapes=[
            pltpu.VMEM((S, D), BF16),
            pltpu.VMEM((HA * 128, S), BF16),
            pltpu.VMEM((HA * VR, S), F32),
            pltpu.VMEM((S, 512), F32),
            pltpu.VMEM((S, 512), F32),
            pltpu.VMEM((1, 512), F32),
            pltpu.VMEM((1, 512), F32),
            pltpu.VMEM((D, S), BF16),
            pltpu.VMEM((S, D), F32),
            pltpu.VMEM((S, 128), F32),
            pltpu.VMEM((3, D, HB, DHB), BF16),
            pltpu.VMEM((3, D, HB * DHB), BF16),
            pltpu.VMEM((HB * DHB, D), BF16),
            pltpu.SemaphoreType.DMA((4,)),
        ],
        compiler_params=pltpu.CompilerParams(vmem_limit_bytes=110 * 2**20),
    )(
        A_x.reshape(S, D), A_wqkv, A_wo, B_mem0.reshape(M, D), gate_w.reshape(1, D),
        B_Wq, B_Wk, B_Wv, B_Wo.reshape(HB * DHB, D),
    )
    return out.reshape(Bn, S, D)
```

```python
import functools

import jax
import jax.numpy as jnp
import jax.experimental.pallas as pl
import jax.experimental.pallas.tpu as pltpu

G = 2
LAGS = (1, 2, 4)
BK = 128
BQ = 512


def APLAN(npos, n):
    return [[] for _ in range(npos - 4)] + [list(range(n * i // 4, n * (i + 1) // 4)) for i in range(4)]


FLAGS = None
SKIP = ()
LATE = False
RLAG = 2
LOG2E = 1.4426950408889634
F32 = jnp.float32
BF16 = jnp.bfloat16
U32 = jnp.uint32
NN = (((1,), (0,)), ((), ()))
NT = (((1,), (1,)), ((), ()))
TN = (((0,), (0,)), ((), ()))


def _pk(x):
    return pltpu.bitcast(x.astype(BF16), U32)


def _unpk(x):
    return pltpu.bitcast(x, BF16)


def _dot(a, b, dims=NN):
    return jax.lax.dot_general(a, b, dims, preferred_element_type=F32)


def _make_kernel(S, D, HA, HB, DHB, M, SEG):
    DHA = D // HA
    NSEG = S // SEG
    L = M + SEG
    NQ = S // BQ
    NK = S // BK
    NU = HA * NQ
    GH = 128 // DHA
    VR = DHA + 8
    NG = HB // G
    SPQ = NSEG // NQ
    assert 2 * SPQ == HA
    RL = 16
    NRL = D // RL

    def kernel(x_hbm, wqkv_hbm, woa_hbm, mem0_ref, gw_ref,
               wq3_hbm, wk3_hbm, wv3_hbm, wob_hbm,
               out_hbm,
               x_ref, wqkv_ref, woa_ref,
               ka_ref, qm_ref, vt_ref, sa_ref, sb_ref, ma_ref, mb_ref, ot_ref,
               b_ref, g_ref, o_ref,
               w3_ref, wqkvb_ref, wob_stage, wob_ref, isems, osems):
        cp_wqkv = pltpu.make_async_copy(wqkv_hbm, wqkv_ref, isems.at[0])
        cp_x = [pltpu.make_async_copy(x_hbm.at[i * BQ:(i + 1) * BQ], x_ref.at[i * BQ:(i + 1) * BQ],
                                      isems.at[1 + i]) for i in range(NQ)]
        cp_w3 = [pltpu.make_async_copy(src, w3_ref.at[t], isems.at[1 + NQ + t])
                 for t, src in enumerate((wq3_hbm, wk3_hbm, wv3_hbm))]
        cp_wob = pltpu.make_async_copy(wob_hbm, wob_stage, isems.at[4 + NQ])
        cp_woa = pltpu.make_async_copy(woa_hbm, woa_ref, isems.at[5 + NQ])
        for c in [cp_wqkv] + cp_x:
            c.start()
        if not LATE:
            for c in cp_w3 + [cp_wob, cp_woa]:
                c.start()

        def fill(i, _):
            qm_ref[pl.ds(pl.multiple_of(i * 64, 64), 64), :] = jnp.zeros((64, S), U32)
            vt_ref[pl.ds(pl.multiple_of(i * VR + DHA, 8), VR - DHA), :] = jnp.ones((VR - DHA, S), F32)
            return 0
        if 'fill' not in SKIP: jax.lax.fori_loop(0, HA, fill, 0)

        cp_wqkv.wait()
        if LATE:
            for c in cp_w3 + [cp_wob, cp_woa]:
                c.start()
        wq_t = wqkv_ref[:, 0:D].astype(F32).T
        wv_t = wqkv_ref[:, 2 * D:3 * D].astype(F32).T
        gw = jnp.broadcast_to(gw_ref[...], (128, D))
        qscale = (DHA ** -0.5) * LOG2E

        def relayout(t, r):
            d0 = r * RL
            u = pltpu.bitcast(w3_ref[t, d0:d0 + RL, :, :], jnp.uint32)
            tt = jnp.swapaxes(u, 0, 1)
            for hp in range(HB // 2):
                ab = tt[hp]
                lo = _pk(pltpu.bitcast(ab << 16, F32))
                hi = _pk(pltpu.bitcast(ab & jnp.uint32(0xFFFF0000), F32))
                wqkvb_ref[t, d0 // 2:(d0 + RL) // 2, (2 * hp) * DHB:(2 * hp + 1) * DHB] = lo
                wqkvb_ref[t, d0 // 2:(d0 + RL) // 2, (2 * hp + 1) * DHB:(2 * hp + 2) * DHB] = hi

        for i in range(NQ):
            rows = slice(i * BQ, (i + 1) * BQ)
            cp_x[i].wait()
            if RLAG <= i <= RLAG + 2:
                cp_w3[i - RLAG].wait()
            xb = x_ref[rows, :]
            ka_ref[i * BQ // 2:(i + 1) * BQ // 2, :] = _pk(_dot(xb, wqkv_ref[:, D:2 * D]))
            qt = _pk(_dot(wq_t, xb, NT) * qscale)
            for h in range(HA):
                j = h % GH
                qm_ref[(h * 128 + j * DHA) // 2:(h * 128 + (j + 1) * DHA) // 2, rows] = qt[h * DHA // 2:(h + 1) * DHA // 2]
            vt = _dot(wv_t, xb, NT)
            for h in range(HA):
                vt_ref[h * VR:h * VR + DHA, rows] = vt[h * DHA:(h + 1) * DHA]
            g_ref[rows, :] = jax.nn.sigmoid(_dot(xb, gw, NT))
            if RLAG <= i <= RLAG + 2 and 'rl' not in SKIP:
                for r in range(NRL):
                    relayout(i - RLAG, r)
        rest = list(range(max(NQ - RLAG, 0), 3))

        def qcols(u):
            return pl.ds(pl.multiple_of((u // HA) * BQ, BQ), BQ)

        def s_chunk(u, c, buf):
            h = u % HA
            qm = _unpk(qm_ref[pl.ds(pl.multiple_of(h * 64, 64), 64), qcols(u)])
            kk = _unpk(ka_ref[c * BK // 2:(c + 1) * BK // 2, pl.ds(pl.multiple_of((h // GH) * 128, 128), 128)])
            st = _dot(kk, qm)
            buf[c * BK:(c + 1) * BK, :] = st
            return jnp.max(st.reshape(BK // 8, 8, BQ), axis=0)

        def phase_tasks(u_s, buf_s, m_s, u_p, buf_p, m_p):
            st = {}
            hp = u_p % HA
            r0 = pl.multiple_of(hp * VR, 8)

            def chunk(c):
                def f():
                    if c == 0:
                        st['m'] = m_p[...]
                        st['ot'] = jnp.zeros((VR, BQ), F32)
                        st['mx8'] = None
                    mc = s_chunk(u_s, c, buf_s)
                    st['mx8'] = mc if st['mx8'] is None else jnp.maximum(st['mx8'], mc)
                    p = jnp.exp2(buf_p[c * BK:(c + 1) * BK, :] - st['m'])
                    st['ot'] = st['ot'] + _dot(vt_ref[pl.ds(r0, VR), c * BK:(c + 1) * BK], p)
                    if c == NK - 1:
                        m_s[...] = jnp.max(st['mx8'], axis=0, keepdims=True)
                        ot = st['ot']
                        ot_ref[pl.ds(pl.multiple_of(hp * DHA, DHA), DHA), qcols(u_p)] = (
                            ot[:DHA] / ot[DHA:DHA + 1]).astype(BF16)
                return f
            return [chunk(c) for c in range(NK)]

        for t in rest:
            cp_w3[t].wait()
        mx8 = None
        for c in range(NK):
            mc = s_chunk(0, c, sa_ref)
            mx8 = mc if mx8 is None else jnp.maximum(mx8, mc)
        ma_ref[...] = jnp.max(mx8, axis=0, keepdims=True)
        for t in rest:
            for r in range(NRL):
                relayout(t, r)
        cp_wob.wait()

        def pack_wob(i, _):
            wob_ref[pl.ds(pl.multiple_of(i * 128, 128), 128), :] = _pk(
                wob_stage[pl.ds(pl.multiple_of(i * 256, 256), 256), :])
            return 0
        jax.lax.fori_loop(0, HB * DHB // 256, pack_wob, 0)
        cp_woa.wait()

        row = jax.lax.broadcasted_iota(jnp.int32, (L, L), 0)
        col = jax.lax.broadcasted_iota(jnp.int32, (L, L), 1)
        allowed = (row >= SEG) | (col >= SEG) | (col <= row)
        bscale = (DHB ** -0.5) * LOG2E
        lS, lPV, lP = LAGS

        def step(s, mem):
            rows = pl.ds(pl.multiple_of(s * SEG, SEG), SEG)
            h = jnp.concatenate([x_ref[rows, :].astype(F32), mem], axis=0)

            def qkv(g):
                cs = slice(g * G * DHB, (g + 1) * G * DHB)
                return tuple(_dot(h, _unpk(wqkvb_ref[t, :, cs])) for t in range(3))

            def attn1(q, k, v):
                ps = []
                for j in range(G):
                    hs = slice(j * DHB, (j + 1) * DHB)
                    sc = _dot(q[:, hs], k[:, hs], NT) * bscale
                    sc = jnp.where(allowed, sc, -1e30)
                    m = jnp.max(sc, axis=1, keepdims=True)
                    p = jnp.exp2(sc - m)
                    l = jnp.sum(p, axis=1, keepdims=True)
                    ps.append((p, pl.reciprocal(l, approx=True)))
                return ps

            def attn2(ps, v):
                os_ = []
                for j in range(G):
                    hs = slice(j * DHB, (j + 1) * DHB)
                    p, rl = ps[j]
                    os_.append(_dot(p, v[:, hs]) * rl)
                return jnp.concatenate(os_, axis=1)

            acc = jnp.zeros((L, D), F32)
            QKV, PS, OG = {}, {}, {}
            u0 = 2 * s
            u1 = u0 + 1
            u2 = jnp.minimum(u0 + 2, NU - 1)
            atasks = (phase_tasks(u1, sb_ref, mb_ref, u0, sa_ref, ma_ref)
                      + phase_tasks(u2, sa_ref, ma_ref, u1, sb_ref, mb_ref))
            plan = APLAN(NG + lP, len(atasks))
            for g in range(NG + lP):
                for ti in plan[g]:
                    atasks[ti]()
                if g < NG:
                    QKV[g] = qkv(g)
                if 0 <= g - lS < NG:
                    PS[g - lS] = attn1(*QKV[g - lS])
                if 0 <= g - lPV < NG:
                    OG[g - lPV] = attn2(PS[g - lPV], QKV[g - lPV][2])
                if 0 <= g - lP < NG:
                    gg = g - lP
                    acc = acc + _dot(OG[gg], _unpk(wob_ref[gg * G * DHB // 2:(gg + 1) * G * DHB // 2, :]))
            b_ref[rows, :] = acc[:SEG]
            return acc[SEG:]

        def out_copy(q):
            rows = pl.ds(pl.multiple_of(q * BQ, BQ), BQ)
            return pltpu.make_async_copy(o_ref.at[rows], out_hbm.at[rows], osems.at[q])

        def qblock(q, mem):
            if 'main' not in SKIP: mem = jax.lax.fori_loop(q * SPQ, (q + 1) * SPQ, step, mem)
            rows = pl.ds(pl.multiple_of(q * BQ, BQ), BQ)
            a = _dot(ot_ref[:, rows], woa_ref[...], TN)
            a = a.astype(BF16).astype(F32)
            b = b_ref[rows, :].astype(BF16).astype(F32)
            g = g_ref[rows, :]
            g = jnp.concatenate([g] * (D // 128), axis=1)
            o_ref[rows, :] = (g * a + (1.0 - g) * b).astype(o_ref.dtype)
            out_copy(q).start()
            return mem

        jax.lax.fori_loop(0, NQ, qblock, mem0_ref[...].astype(F32))
        for q in range(NQ):
            out_copy(q).wait()

    return kernel


@functools.partial(jax.jit, static_argnames=("B_seg_len",))
def pallas_gated_mix__mha_block__memory_aug_recurrent_mem_tr__prompt_kernel(
    A_x, A_wqkv, A_wo, B_x, B_mem0, B_Wq, B_Wk, B_Wv, B_Wo, B_seg_len, gate_w,
):
    del B_x
    Bn, S, D = A_x.shape
    assert Bn == 1
    HA = 32
    _, HB, DHB = B_Wq.shape
    M = B_mem0.shape[1]
    SEG = int(B_seg_len)
    DHA = D // HA
    VR = DHA + 8
    NQ = S // BQ
    kernel = _make_kernel(S, D, HA, HB, DHB, M, SEG)
    vmem = pl.BlockSpec(memory_space=pltpu.VMEM)
    hbm = pl.BlockSpec(memory_space=pl.ANY)
    out = pl.pallas_call(
        kernel,
        out_shape=jax.ShapeDtypeStruct((S, D), A_x.dtype),
        in_specs=[hbm, hbm, hbm, vmem, vmem, hbm, hbm, hbm, hbm],
        out_specs=hbm,
        scratch_shapes=[
            pltpu.VMEM((S, D), BF16),
            pltpu.VMEM((D, 3 * D), BF16),
            pltpu.VMEM((D, D), BF16),
            pltpu.VMEM((S // 2, D), U32),
            pltpu.VMEM((HA * 64, S), U32),
            pltpu.VMEM((HA * VR, S), F32),
            pltpu.VMEM((S, BQ), F32),
            pltpu.VMEM((S, BQ), F32),
            pltpu.VMEM((1, BQ), F32),
            pltpu.VMEM((1, BQ), F32),
            pltpu.VMEM((D, S), BF16),
            pltpu.VMEM((S, D), F32),
            pltpu.VMEM((S, 128), F32),
            pltpu.VMEM((S, D), A_x.dtype),
            pltpu.VMEM((3, D, HB, DHB), BF16),
            pltpu.VMEM((3, D // 2, HB * DHB), U32),
            pltpu.VMEM((HB * DHB, D), BF16),
            pltpu.VMEM((HB * DHB // 2, D), U32),
            pltpu.SemaphoreType.DMA((NQ + 6,)),
            pltpu.SemaphoreType.DMA((NQ,)),
        ],
        compiler_params=pltpu.CompilerParams(vmem_limit_bytes=110 * 2**20, flags=FLAGS),
    )(
        A_x.reshape(S, D), A_wqkv, A_wo, B_mem0.reshape(M, D), gate_w.reshape(1, D),
        B_Wq, B_Wk, B_Wv, B_Wo.reshape(HB * DHB, D),
    )
    return out.reshape(Bn, S, D)
```

```python
import functools

import jax
import jax.numpy as jnp
import jax.experimental.pallas as pl
import jax.experimental.pallas.tpu as pltpu

G = 2
LAGS = (1, 2, 4)
BK = 128
BQ = 512


def APLAN(npos, n):
    return [[] for _ in range(npos - 4)] + [list(range(n * i // 4, n * (i + 1) // 4)) for i in range(4)]


FLAGS = None
N0 = 8
A1W = [None, None, None, None]
A2W = [0, 1, 2, 3]
SKIP = ()
UNR = 1
HOIST = False
RCP = False
PFIRST = False
PVS = 1
PACE = True
XB = 0
LATE = False
RLAG = 2
LOG2E = 1.4426950408889634
F32 = jnp.float32
BF16 = jnp.bfloat16
U32 = jnp.uint32
NN = (((1,), (0,)), ((), ()))
NT = (((1,), (1,)), ((), ()))
TN = (((0,), (0,)), ((), ()))


def _pk(x):
    return pltpu.bitcast(x.astype(BF16), U32)


def _unpk(x):
    return pltpu.bitcast(x, BF16)


def _dot(a, b, dims=NN):
    return jax.lax.dot_general(a, b, dims, preferred_element_type=F32)


def _make_kernel(S, D, HA, HB, DHB, M, SEG):
    DHA = D // HA
    NSEG = S // SEG
    L = M + SEG
    NQ = S // BQ
    NK = S // BK
    NU = HA * NQ
    GH = 128 // DHA
    VR = DHA + 8
    NG = HB // G
    SPQ = NSEG // NQ
    assert 2 * SPQ == HA
    RL = 16
    NRL = D // RL
    WP = D + 8

    def kernel(x_hbm, wqkv_hbm, woa_hbm, mem0_ref, gw_ref,
               wq3_hbm, wk3_hbm, wv3_hbm, wob_hbm,
               out_hbm,
               x_ref, wqkv_ref, woa_ref,
               ka_ref, qm_ref, vt_ref, ma_ref, mb_ref, ot_ref,
               b_ref, g_ref, o_ref,
               w3_ref, wqkvb_ref, wob_stage, wob_ref, isems, osems, *sbufs):
        sa_ref, sb_ref = sbufs[:NK], sbufs[NK:]
        cp_wqkv = pltpu.make_async_copy(wqkv_hbm, wqkv_ref, isems.at[0])
        cp_x = [pltpu.make_async_copy(x_hbm.at[i * BQ:(i + 1) * BQ], x_ref.at[i * BQ:(i + 1) * BQ],
                                      isems.at[1 + i]) for i in range(NQ)]
        cp_w3 = [pltpu.make_async_copy(src, w3_ref.at[t], isems.at[1 + NQ + t])
                 for t, src in enumerate((wq3_hbm, wk3_hbm, wv3_hbm))]
        cp_wob = pltpu.make_async_copy(wob_hbm, wob_stage, isems.at[4 + NQ])
        cp_woa = pltpu.make_async_copy(woa_hbm, woa_ref, isems.at[5 + NQ])
        for c in [cp_wqkv] + cp_x:
            c.start()
        if not LATE:
            for c in cp_w3 + [cp_wob, cp_woa]:
                c.start()

        def fill(i, _):
            qm_ref[pl.ds(pl.multiple_of(i * 64, 64), 64), :] = jnp.zeros((64, S), U32)
            vt_ref[pl.ds(pl.multiple_of(i * VR + DHA, 8), VR - DHA), :] = jnp.ones((VR - DHA, S), F32)
            return 0
        if 'fill' not in SKIP: jax.lax.fori_loop(0, HA, fill, 0)

        cp_wqkv.wait()
        wq_t = wqkv_ref[:, 0:D].astype(F32).T
        wv_t = wqkv_ref[:, 2 * D:3 * D].astype(F32).T
        gw = jnp.broadcast_to(gw_ref[...], (128, D))
        qscale = (DHA ** -0.5) * LOG2E

        def zero_after(tok):
            z = pltpu.bitcast(jnp.abs(tok), U32) >> 31
            return jnp.concatenate([z, z], axis=0)

        def relayout(t, r, tok):
            if tok is None or not PACE:
                lo, hi = jnp.uint32(0xFFFF), jnp.uint32(0xFFFF0000)
            else:
                z = zero_after(tok)
                lo, hi = z | jnp.uint32(0xFFFF), z | jnp.uint32(0xFFFF0000)
            for j in range(r * RL // 2, (r + 1) * RL // 2):
                a = pltpu.bitcast(w3_ref[t, 2 * j], U32)
                b = pltpu.bitcast(w3_ref[t, 2 * j + 1], U32)
                e = (a & lo) | (b << 16)
                o = (a >> 16) | (b & hi)
                for i in range(HB // 16):
                    wqkvb_ref[t, pl.ds(8 * i * WP + j, 8, stride=WP), :] = e[8 * i:8 * i + 8]
                    wqkvb_ref[t, pl.ds(8 * i * WP + D // 2 + j, 8, stride=WP), :] = o[8 * i:8 * i + 8]

        def wslab(t, h):
            base = (h // 2) * WP + (h % 2) * (D // 2)
            return wqkvb_ref[t, base:base + D // 2, :]

        def pack_wob(r, tok):
            wob_ref[r * 64:(r + 1) * 64, :] = _pk(wob_stage[r * 128:(r + 1) * 128, :])

        def weight_tasks(t):
            if 'rl' in SKIP:
                return [lambda tok: (cp_w3[t].wait() if t < 3 else cp_wob.wait())]
            if t < 3:
                return [lambda tok: cp_w3[t].wait()] + [functools.partial(relayout, t, r) for r in range(NRL)]
            return [lambda tok: cp_wob.wait()] + [functools.partial(pack_wob, r) for r in range(HB * DHB // 128)]

        def interleave(main, side):
            n, k = len(main), len(side)
            tok = None
            for i, f in enumerate(main):
                for g in side[(k * i) // n:(k * (i + 1)) // n]:
                    g(tok)
                tok = f()

        def proj_tasks(i):
            rows = slice(i * BQ, (i + 1) * BQ)
            PR = 128
            tasks = []

            def k_piece(j):
                xb = x_ref[i * BQ + j * PR:i * BQ + (j + 1) * PR, :]
                kk = _dot(xb, wqkv_ref[:, D:2 * D])
                ka_ref[(i * BQ + j * PR) // 2:(i * BQ + (j + 1) * PR) // 2, :] = _pk(kk)
                g_ref[i * BQ + j * PR:i * BQ + (j + 1) * PR, :] = jax.nn.sigmoid(_dot(xb, gw, NT))
                return kk[0:8, 0:128]

            def q_piece(j):
                qf = _dot(wq_t[j * PR:(j + 1) * PR], x_ref[rows, :], NT)
                qt = _pk(qf * qscale)
                for hh in range(PR // DHA):
                    h = j * (PR // DHA) + hh
                    jj = h % GH
                    qm_ref[(h * 128 + jj * DHA) // 2:(h * 128 + (jj + 1) * DHA) // 2, rows] = (
                        qt[hh * DHA // 2:(hh + 1) * DHA // 2])
                return qf[0:8, 0:128]

            def v_piece(j):
                vt = _dot(wv_t[j * PR:(j + 1) * PR], x_ref[rows, :], NT)
                for hh in range(PR // DHA):
                    h = j * (PR // DHA) + hh
                    vt_ref[h * VR:h * VR + DHA, rows] = vt[hh * DHA:(hh + 1) * DHA]
                return vt[0:8, 0:128]

            for j in range(BQ // PR):
                tasks.append(functools.partial(k_piece, j))
            for j in range(D // PR):
                tasks.append(functools.partial(q_piece, j))
                tasks.append(functools.partial(v_piece, j))
            return tasks

        for i in range(NQ):
            cp_x[i].wait()
            interleave(proj_tasks(i), weight_tasks(A1W[i]) if A1W[i] is not None else [])

        def qcols(u):
            return pl.ds(pl.multiple_of((u // HA) * BQ, BQ), BQ)

        def load_qm(u):
            h = u % HA
            return _unpk(qm_ref[pl.ds(pl.multiple_of(h * 64, 64), 64), qcols(u)])

        def s_chunk(u, c, buf, qm=None):
            h = u % HA
            if qm is None:
                qm = load_qm(u)
            kk = _unpk(ka_ref[c * BK // 2:(c + 1) * BK // 2, pl.ds(pl.multiple_of((h // GH) * 128, 128), 128)])
            st = _dot(kk, qm)
            buf[c][...] = st
            return jnp.max(st.reshape(BK // 8, 8, BQ), axis=0)

        def phase_tasks(u_s, buf_s, m_s, u_p, buf_p, m_p):
            st = {}
            hp = u_p % HA
            r0 = pl.multiple_of(hp * VR, 8)

            def chunk(c):
                def f():
                    if c == 0:
                        st['m'] = m_p[...]
                        st['ot'] = jnp.zeros((VR, BQ), F32)
                        st['mx8'] = None
                        st['qm'] = load_qm(u_s) if HOIST else None
                    def do_s():
                        mc = s_chunk(u_s, c, buf_s, st['qm'])
                        st['mx8'] = mc if st['mx8'] is None else jnp.maximum(st['mx8'], mc)
                        return mc

                    def do_p():
                        for cc in range(c * PVS, (c + 1) * PVS):
                            ks = slice(cc * BK // PVS, (cc + 1) * BK // PVS)
                            p = jnp.exp2(buf_p[c][(cc - c * PVS) * BK // PVS:(cc - c * PVS + 1) * BK // PVS, :] - st['m'])
                            st['ot'] = st['ot'] + _dot(vt_ref[pl.ds(r0, VR), ks], p)
                    if PFIRST:
                        do_p()
                        mc = do_s()
                    else:
                        mc = do_s()
                        do_p()
                    if c == NK - 1:
                        m_s[...] = jnp.max(st['mx8'], axis=0, keepdims=True)
                        ot = st['ot']
                        if RCP:
                            l = ot[DHA:DHA + 1]
                            r = pl.reciprocal(l, approx=True)
                            r = r * (2.0 - l * r)
                            o = ot[:DHA] * r
                        else:
                            o = ot[:DHA] / ot[DHA:DHA + 1]
                        ot_ref[pl.ds(pl.multiple_of(hp * DHA, DHA), DHA), qcols(u_p)] = o.astype(BF16)
                    return mc[:, 0:128]
                return f
            return [chunk(c) for c in range(NK)]

        mx8 = None
        for c in range(NK):
            mc = s_chunk(0, c, sa_ref)
            mx8 = mc if mx8 is None else jnp.maximum(mx8, mc)
        ma_ref[...] = jnp.max(mx8, axis=0, keepdims=True)

        for j in range(N0 // 2):
            u0 = 2 * j
            interleave(phase_tasks(u0 + 1, sb_ref, mb_ref, u0, sa_ref, ma_ref)
                       + phase_tasks(u0 + 2, sa_ref, ma_ref, u0 + 1, sb_ref, mb_ref),
                       weight_tasks(A2W[j]) if A2W[j] is not None else [])
        for t in range(4):
            if t not in A1W and t not in A2W[:N0 // 2]:
                for f in weight_tasks(t):
                    f(None)
        cp_woa.wait()

        row = jax.lax.broadcasted_iota(jnp.int32, (L, L), 0)
        col = jax.lax.broadcasted_iota(jnp.int32, (L, L), 1)
        allowed = (row >= SEG) | (col >= SEG) | (col <= row)
        bscale = (DHB ** -0.5) * LOG2E
        lS, lPV, lP = LAGS

        def step(s, mem, with_a=True):
            rows = pl.ds(pl.multiple_of(s * SEG, SEG), SEG)
            h = jnp.concatenate([x_ref[rows, :].astype(F32), mem], axis=0)

            def qkv(g):
                return tuple(
                    _dot(h, _unpk(jnp.concatenate([wslab(t, hh) for hh in range(g * G, (g + 1) * G)], axis=1)))
                    for t in range(3))

            def attn1(q, k, v):
                ps = []
                for j in range(G):
                    hs = slice(j * DHB, (j + 1) * DHB)
                    sc = _dot(q[:, hs], k[:, hs], NT) * bscale
                    sc = jnp.where(allowed, sc, -1e30)
                    m = jnp.max(sc, axis=1, keepdims=True)
                    p = jnp.exp2(sc - m)
                    l = jnp.sum(p, axis=1, keepdims=True)
                    ps.append((p, pl.reciprocal(l, approx=True)))
                return ps

            def attn2(ps, v):
                os_ = []
                for j in range(G):
                    hs = slice(j * DHB, (j + 1) * DHB)
                    p, rl = ps[j]
                    os_.append(_dot(p, v[:, hs]) * rl)
                return jnp.concatenate(os_, axis=1)

            acc = jnp.zeros((L, D), F32)
            QKV, PS, OG = {}, {}, {}
            if with_a:
                u0 = 2 * s + N0
                u1 = u0 + 1
                u2 = jnp.minimum(u0 + 2, NU - 1)
                atasks = (phase_tasks(u1, sb_ref, mb_ref, u0, sa_ref, ma_ref)
                          + phase_tasks(u2, sa_ref, ma_ref, u1, sb_ref, mb_ref))
                plan = APLAN(NG + lP, len(atasks))
            else:
                plan = [[] for _ in range(NG + lP)]
            for g in range(NG + lP):
                for ti in plan[g]:
                    atasks[ti]()
                if g < NG:
                    QKV[g] = qkv(g)
                if 0 <= g - lS < NG:
                    PS[g - lS] = attn1(*QKV[g - lS])
                if 0 <= g - lPV < NG:
                    OG[g - lPV] = attn2(PS[g - lPV], QKV[g - lPV][2])
                if 0 <= g - lP < NG:
                    gg = g - lP
                    acc = acc + _dot(OG[gg], _unpk(wob_ref[gg * G * DHB // 2:(gg + 1) * G * DHB // 2, :]))
            b_ref[rows, :] = acc[:SEG]
            return acc[SEG:]

        def out_copy(q):
            rows = pl.ds(pl.multiple_of(q * BQ, BQ), BQ)
            return pltpu.make_async_copy(o_ref.at[rows], out_hbm.at[rows], osems.at[q])

        def mix(q):
            rows = pl.ds(pl.multiple_of(q * BQ, BQ), BQ)
            a = _dot(ot_ref[:, rows], woa_ref[...], TN)
            b = b_ref[rows, :]
            g = g_ref[rows, :]
            g = jnp.concatenate([g] * (D // 128), axis=1)
            o_ref[rows, :] = (g * a + (1.0 - g) * b).astype(o_ref.dtype)
            out_copy(q).start()

        if 'mix' in SKIP:
            def mix(q):
                if 'nocopy' not in SKIP: out_copy(q).start()
        NJ = NSEG - N0 // 2

        def qblock(q, mem):
            def steps(i, mem):
                for j in range(UNR):
                    mem = step(i * UNR + j, mem)
                return mem
            if 'main' not in SKIP: mem = jax.lax.fori_loop(q * (SPQ // UNR), jnp.minimum((q + 1) * SPQ, NJ) // UNR, steps, mem)
            if N0:
                pl.when(q < NQ - 1)(lambda: mix(q))
            else:
                mix(q)
            return mem

        mem = jax.lax.fori_loop(0, NQ, qblock, mem0_ref[...].astype(F32))
        if N0:
            if 'bonly' not in SKIP: jax.lax.fori_loop(NJ - XB, NSEG, functools.partial(step, with_a=False), mem)
            mix(NQ - 1)
        if 'nocopy' not in SKIP:
            for q in range(NQ):
                out_copy(q).wait()

    return kernel


@functools.partial(jax.jit, static_argnames=("B_seg_len",))
def pallas_gated_mix__mha_block__memory_aug_recurrent_mem_tr__prompt_kernel(
    A_x, A_wqkv, A_wo, B_x, B_mem0, B_Wq, B_Wk, B_Wv, B_Wo, B_seg_len, gate_w,
):
    del B_x
    Bn, S, D = A_x.shape
    assert Bn == 1
    HA = 32
    _, HB, DHB = B_Wq.shape
    M = B_mem0.shape[1]
    SEG = int(B_seg_len)
    DHA = D // HA
    VR = DHA + 8
    NQ = S // BQ
    kernel = _make_kernel(S, D, HA, HB, DHB, M, SEG)
    vmem = pl.BlockSpec(memory_space=pltpu.VMEM)
    hbm = pl.BlockSpec(memory_space=pl.ANY)
    out = pl.pallas_call(
        kernel,
        out_shape=jax.ShapeDtypeStruct((S, D), A_x.dtype),
        in_specs=[hbm, hbm, hbm, vmem, vmem, hbm, hbm, hbm, hbm],
        out_specs=hbm,
        scratch_shapes=[
            pltpu.VMEM((S, D), BF16),
            pltpu.VMEM((D, 3 * D), BF16),
            pltpu.VMEM((D, D), BF16),
            pltpu.VMEM((S // 2, D), U32),
            pltpu.VMEM((HA * 64, S), U32),
            pltpu.VMEM((HA * VR, S), F32),
            pltpu.VMEM((1, BQ), F32),
            pltpu.VMEM((1, BQ), F32),
            pltpu.VMEM((D, S), BF16),
            pltpu.VMEM((S, D), F32),
            pltpu.VMEM((S, 128), F32),
            pltpu.VMEM((S, D), A_x.dtype),
            pltpu.VMEM((3, D, HB, DHB), BF16),
            pltpu.VMEM((3, (HB // 2) * (D + 8), DHB), U32),
            pltpu.VMEM((HB * DHB, D), BF16),
            pltpu.VMEM((HB * DHB // 2, D), U32),
            pltpu.SemaphoreType.DMA((NQ + 6,)),
            pltpu.SemaphoreType.DMA((NQ,)),
        ] + [pltpu.VMEM((BK, BQ), F32) for _ in range(2 * (S // BK))],
        compiler_params=pltpu.CompilerParams(vmem_limit_bytes=110 * 2**20, flags=FLAGS),
    )(
        A_x.reshape(S, D), A_wqkv, A_wo, B_mem0.reshape(M, D), gate_w.reshape(1, D),
        B_Wq, B_Wk, B_Wv, B_Wo.reshape(HB * DHB, D),
    )
    return out.reshape(Bn, S, D)
```

```python
import functools

import jax
import jax.numpy as jnp
import jax.experimental.pallas as pl
import jax.experimental.pallas.tpu as pltpu

G = 2
LAGS = (1, 2, 4)
BK = 128
BQ = 512
N0 = 6
MR = 128
UNR = 1


def APLAN(npos, n):
    return [[] for _ in range(npos - 4)] + [[0, 1], [2, 3], list(range(4, 16)), list(range(16, 32))]


SKIP = ()
GATE = 'vpu'
XB = 0
PACE = True
FLAGS = None
LOG2E = 1.4426950408889634
F32 = jnp.float32
BF16 = jnp.bfloat16
U32 = jnp.uint32
NN = (((1,), (0,)), ((), ()))
NT = (((1,), (1,)), ((), ()))
TN = (((0,), (0,)), ((), ()))


def _pk(x):
    return pltpu.bitcast(x.astype(BF16), U32)


def _unpk(x):
    return pltpu.bitcast(x, BF16)


def _dot(a, b, dims=NN):
    return jax.lax.dot_general(a, b, dims, preferred_element_type=F32)


def _interleave(main, side):
    n, k = len(main), len(side)
    tok = None
    for i, f in enumerate(main):
        for g in side[(k * i) // n:(k * (i + 1)) // n]:
            g(tok)
        tok = f()


def _zero_after(tok):
    if tok is None or not PACE:
        return jnp.zeros((8, 128), U32)
    return pltpu.bitcast(jnp.abs(tok), U32) >> 31


def _make_kernel(S, D, HA, HB, DHB, M, SEG):
    DHA = D // HA
    NSEG = S // SEG
    L = M + SEG
    NQ = S // BQ
    NK = S // BK
    NU = HA * NQ
    GH = 128 // DHA
    VR = DHA + 8
    NG = HB // G
    SPQ = NSEG // NQ
    assert 2 * SPQ == HA and N0 % 2 == 0 and N0 >= 6
    WP = D + 8
    RL = 16
    PR = 128

    def kernel(x_hbm, wqkv_hbm, woa_hbm, mem0_ref, gw_ref,
               wq3_hbm, wk3_hbm, wv3_hbm, wob_hbm,
               out_hbm,
               x_ref, wqkv_ref, woa_ref, woap_ref,
               ka_ref, qm_ref, vt_ref, ma_ref, mb_ref, ot_ref,
               b_ref, g_ref, o_ref,
               w3_ref, wqkvb_ref, wob_stage, wob_ref, isems, osems, *sbufs):
        sa_ref, sb_ref = sbufs[:NK], sbufs[NK:]

        def x_copy(i):
            rows = pl.ds(pl.multiple_of(i * BQ, BQ), BQ)
            return pltpu.make_async_copy(x_hbm.at[rows], x_ref.at[rows], isems.at[i])

        def w3_copy(t, src):
            return pltpu.make_async_copy(src, w3_ref.at[t], isems.at[NQ + t])

        cp_wa = [pltpu.make_async_copy(wqkv_hbm.at[:, t * D:(t + 1) * D], wqkv_ref.at[:, t * D:(t + 1) * D],
                                       isems.at[NQ + 6 + t]) for t in range(3)]
        cp_wob = pltpu.make_async_copy(wob_hbm, wob_stage, isems.at[NQ + 4])
        cp_woa = pltpu.make_async_copy(woa_hbm, woa_ref, isems.at[NQ + 5])
        cp_wa[1].start()
        x_copy(0).start()
        x_copy(1).start()
        cp_wa[0].start()
        x_copy(2).start()
        cp_wa[2].start()
        for i in range(3, NQ):
            x_copy(i).start()
        cp_wob.start()
        for t, src in enumerate((wq3_hbm, wk3_hbm, wv3_hbm)):
            w3_copy(t, src).start()
        cp_woa.start()

        gw = gw_ref[...].astype(F32)
        gwb = jnp.broadcast_to(gw_ref[...], (128, D))
        qscale = (DHA ** -0.5) * LOG2E

        def fill(h, tok):
            z = _zero_after(tok)
            qm_ref[pl.ds(pl.multiple_of(h * 64, 64), 64), :] = jnp.tile(z, (8, S // 128))
            one = pltpu.bitcast(z | jnp.uint32(0x3F800000), F32)
            vt_ref[pl.ds(pl.multiple_of(h * VR + DHA, 8), VR - DHA), :] = jnp.tile(one, ((VR - DHA) // 8, S // 128))

        def proj_k(i, _):
            x_copy(i).wait()

            def piece(j):
                def f():
                    rows = pl.ds(pl.multiple_of(i * BQ + j * PR, PR), PR)
                    xb = x_ref[rows, :]
                    kk = _dot(xb, wqkv_ref[:, D:2 * D])
                    ka_ref[pl.ds(pl.multiple_of((i * BQ + j * PR) // 2, PR // 2), PR // 2), :] = _pk(kk)
                    if GATE == 'vpu':
                        z = jnp.sum(xb.astype(F32) * gw, axis=1, keepdims=True)
                        g_ref[rows, :] = jnp.broadcast_to(jax.nn.sigmoid(z), (PR, 128))
                    else:
                        g_ref[rows, :] = jax.nn.sigmoid(_dot(xb, gwb, NT))
                    return kk[0:8, 0:128]
                return f
            hpb = HA // NQ
            _interleave([piece(j) for j in range(BQ // PR)],
                        [functools.partial(fill, i * hpb + hh) for hh in range(hpb)])
            return 0
        cp_wa[1].wait()
        jax.lax.fori_loop(0, NQ, proj_k, 0)

        cp_wa[0].wait()
        cp_wa[2].wait()
        wq_t = wqkv_ref[:, 0:D].astype(F32).T
        wv_t = wqkv_ref[:, 2 * D:3 * D].astype(F32).T

        def proj_qv(i, _):
            cols = pl.ds(pl.multiple_of(i * BQ, BQ), BQ)
            for j in range(D // PR):
                qt = _pk(_dot(wq_t[j * PR:(j + 1) * PR], x_ref[cols, :], NT) * qscale)
                vt = _dot(wv_t[j * PR:(j + 1) * PR], x_ref[cols, :], NT)
                for hh in range(PR // DHA):
                    h = j * (PR // DHA) + hh
                    r0 = (h * 128 + (h % GH) * DHA) // 2
                    qm_ref[r0:r0 + DHA // 2, cols] = qt[hh * DHA // 2:(hh + 1) * DHA // 2]
                    vt_ref[h * VR:h * VR + DHA, cols] = vt[hh * DHA:(hh + 1) * DHA]
            return 0
        jax.lax.fori_loop(0, NQ, proj_qv, 0)

        def qcols(u):
            return pl.ds(pl.multiple_of((u // HA) * BQ, BQ), BQ)

        def s_chunk(u, c, buf):
            h = u % HA
            qm = _unpk(qm_ref[pl.ds(pl.multiple_of(h * 64, 64), 64), qcols(u)])
            kk = _unpk(ka_ref[c * BK // 2:(c + 1) * BK // 2, pl.ds(pl.multiple_of((h // GH) * 128, 128), 128)])
            st = _dot(kk, qm)
            buf[c][...] = st
            return jnp.max(st.reshape(BK // 8, 8, BQ), axis=0)

        def phase_tasks(u_s, buf_s, m_s, u_p, buf_p, m_p):
            st = {}
            hp = u_p % HA
            r0 = pl.multiple_of(hp * VR, 8)

            def chunk(c):
                def f():
                    if c == 0:
                        st['m'] = m_p[...]
                        st['ot'] = jnp.zeros((VR, BQ), F32)
                        st['mx8'] = None
                    mc = s_chunk(u_s, c, buf_s)
                    st['mx8'] = mc if st['mx8'] is None else jnp.maximum(st['mx8'], mc)
                    p = jnp.exp2(buf_p[c][...] - st['m'])
                    st['ot'] = st['ot'] + _dot(vt_ref[pl.ds(r0, VR), c * BK:(c + 1) * BK], p)
                    if c == NK - 1:
                        m_s[...] = jnp.max(st['mx8'], axis=0, keepdims=True)
                        ot = st['ot']
                        ot_ref[pl.ds(pl.multiple_of(hp * (DHA // 2), DHA // 2), DHA // 2), qcols(u_p)] = _pk(
                            ot[:DHA] / ot[DHA:DHA + 1])
                    return mc[:, 0:128]
                return f
            return [chunk(c) for c in range(NK)]

        def pair_tasks(u0):
            u1 = u0 + 1
            u2 = jnp.minimum(u0 + 2, NU - 1)
            return (phase_tasks(u1, sb_ref, mb_ref, u0, sa_ref, ma_ref)
                    + phase_tasks(u2, sa_ref, ma_ref, u1, sb_ref, mb_ref))

        def relayout(t, r, tok):
            z = _zero_after(tok)
            z = jnp.concatenate([z] * (HB // 16), axis=0)
            lo, hi = z | jnp.uint32(0xFFFF), z | jnp.uint32(0xFFFF0000)
            for j in range(r * RL // 2, (r + 1) * RL // 2):
                a = pltpu.bitcast(w3_ref[t, 2 * j], U32)
                b = pltpu.bitcast(w3_ref[t, 2 * j + 1], U32)
                e = (a & lo) | (b << 16)
                o = (a >> 16) | (b & hi)
                for i in range(HB // 16):
                    wqkvb_ref[t, pl.ds(8 * i * WP + j, 8, stride=WP), :] = e[8 * i:8 * i + 8]
                    wqkvb_ref[t, pl.ds(8 * i * WP + D // 2 + j, 8, stride=WP), :] = o[8 * i:8 * i + 8]

        def pack_wob(r, tok):
            wob_ref[r * 64:(r + 1) * 64, :] = _pk(wob_stage[r * 128:(r + 1) * 128, :])

        def wslab(t, h):
            base = (h // 2) * WP + (h % 2) * (D // 2)
            return wqkvb_ref[t, base:base + D // 2, :]

        cp_wob.wait()
        first = {'mx8': None}

        def first_chunk(c):
            def f():
                mc = s_chunk(0, c, sa_ref)
                first['mx8'] = mc if first['mx8'] is None else jnp.maximum(first['mx8'], mc)
                return mc[:, 0:128]
            return f
        _interleave([first_chunk(c) for c in range(NK)],
                    [functools.partial(pack_wob, r) for r in range(HB * DHB // 128)])
        ma_ref[...] = jnp.max(first['mx8'], axis=0, keepdims=True)

        def ahead(j, _):
            t = jnp.minimum(j, 2)

            @pl.when(j < 3)
            def _():
                w3_copy(t, wq3_hbm).wait()
            _interleave(pair_tasks(2 * j), [functools.partial(relayout, t, r) for r in range(D // RL)])
            return 0
        jax.lax.fori_loop(0, N0 // 2, ahead, 0)
        cp_woa.wait()
        woap_ref[...] = _pk(woa_ref[...])

        row = jax.lax.broadcasted_iota(jnp.int32, (L, L), 0)
        col = jax.lax.broadcasted_iota(jnp.int32, (L, L), 1)
        allowed = (row >= SEG) | (col >= SEG) | (col <= row)
        bscale = (DHB ** -0.5) * LOG2E
        lS, lPV, lP = LAGS

        def step(s, mem, with_a=True):
            rows = pl.ds(pl.multiple_of(s * SEG, SEG), SEG)
            h = jnp.concatenate([x_ref[rows, :].astype(F32), mem], axis=0)

            def qkv(g):
                return tuple(
                    _dot(h, _unpk(jnp.concatenate([wslab(t, hh) for hh in range(g * G, (g + 1) * G)], axis=1)))
                    for t in range(3))

            def attn1(q, k, v):
                ps = []
                for j in range(G):
                    hs = slice(j * DHB, (j + 1) * DHB)
                    sc = _dot(q[:, hs], k[:, hs], NT) * bscale
                    sc = jnp.where(allowed, sc, -1e30)
                    m = jnp.max(sc, axis=1, keepdims=True)
                    p = jnp.exp2(sc - m)
                    l = jnp.sum(p, axis=1, keepdims=True)
                    ps.append((p, pl.reciprocal(l, approx=True)))
                return ps

            def attn2(ps, v):
                os_ = []
                for j in range(G):
                    hs = slice(j * DHB, (j + 1) * DHB)
                    p, rl = ps[j]
                    os_.append(_dot(p, v[:, hs]) * rl)
                return jnp.concatenate(os_, axis=1)

            acc = jnp.zeros((L, D), F32)
            QKV, PS, OG = {}, {}, {}
            if with_a:
                atasks = pair_tasks(2 * s + N0)
                plan = APLAN(NG + lP, len(atasks))
            else:
                plan = [[] for _ in range(NG + lP)]
            for g in range(NG + lP):
                for ti in plan[g]:
                    atasks[ti]()
                if g < NG:
                    QKV[g] = qkv(g)
                if 0 <= g - lS < NG:
                    PS[g - lS] = attn1(*QKV[g - lS])
                if 0 <= g - lPV < NG:
                    OG[g - lPV] = attn2(PS[g - lPV], QKV[g - lPV][2])
                if 0 <= g - lP < NG:
                    gg = g - lP
                    acc = acc + _dot(OG[gg], _unpk(wob_ref[gg * G * DHB // 2:(gg + 1) * G * DHB // 2, :]))
            b_ref[rows, :] = acc[:SEG]
            return acc[SEG:]

        def out_copy(q):
            rows = pl.ds(pl.multiple_of(q * BQ, BQ), BQ)
            return pltpu.make_async_copy(o_ref.at[rows], out_hbm.at[rows], osems.at[q])

        def mix(q):
            for j in range(BQ // MR):
                rows = pl.ds(pl.multiple_of(q * BQ + j * MR, MR), MR)
                a = _dot(_unpk(ot_ref[:, rows]), _unpk(woap_ref[...]), TN)
                g = g_ref[rows, :]
                g = jnp.concatenate([g] * (D // 128), axis=1)
                o_ref[rows, :] = (g * a + (1.0 - g) * b_ref[rows, :]).astype(o_ref.dtype)
            out_copy(q).start()

        NJ = NSEG - N0 // 2

        def steps(i, mem):
            for j in range(UNR):
                mem = step(i * UNR + j, mem)
            return mem

        def qblock(q, mem):
            if 'main' not in SKIP:
                mem = jax.lax.fori_loop(q * (SPQ // UNR), jnp.minimum((q + 1) * SPQ, NJ) // UNR, steps, mem)
            if 'mix' not in SKIP:
                pl.when(q < NQ - 1)(lambda: mix(q))
            return mem

        mem = jax.lax.fori_loop(0, NQ, qblock, mem0_ref[...].astype(F32))
        if 'bonly' not in SKIP:
            jax.lax.fori_loop(NJ - XB, NSEG, functools.partial(step, with_a=False), mem)
        if 'mix' not in SKIP:
            mix(NQ - 1)
            for q in range(NQ):
                out_copy(q).wait()

    return kernel


@functools.partial(jax.jit, static_argnames=("B_seg_len",))
def pallas_gated_mix__mha_block__memory_aug_recurrent_mem_tr__prompt_kernel(
    A_x, A_wqkv, A_wo, B_x, B_mem0, B_Wq, B_Wk, B_Wv, B_Wo, B_seg_len, gate_w,
):
    del B_x
    Bn, S, D = A_x.shape
    assert Bn == 1
    HA = 32
    _, HB, DHB = B_Wq.shape
    M = B_mem0.shape[1]
    SEG = int(B_seg_len)
    DHA = D // HA
    VR = DHA + 8
    NQ = S // BQ
    kernel = _make_kernel(S, D, HA, HB, DHB, M, SEG)
    vmem = pl.BlockSpec(memory_space=pltpu.VMEM)
    hbm = pl.BlockSpec(memory_space=pl.ANY)
    out = pl.pallas_call(
        kernel,
        out_shape=jax.ShapeDtypeStruct((S, D), A_x.dtype),
        in_specs=[hbm, hbm, hbm, vmem, vmem, hbm, hbm, hbm, hbm],
        out_specs=hbm,
        scratch_shapes=[
            pltpu.VMEM((S, D), BF16),
            pltpu.VMEM((D, 3 * D), BF16),
            pltpu.VMEM((D, D), BF16),
            pltpu.VMEM((D // 2, D), U32),
            pltpu.VMEM((S // 2, D), U32),
            pltpu.VMEM((HA * 64, S), U32),
            pltpu.VMEM((HA * VR, S), F32),
            pltpu.VMEM((1, BQ), F32),
            pltpu.VMEM((1, BQ), F32),
            pltpu.VMEM((D // 2, S), U32),
            pltpu.VMEM((S, D), F32),
            pltpu.VMEM((S, 128), F32),
            pltpu.VMEM((S, D), A_x.dtype),
            pltpu.VMEM((3, D, HB, DHB), BF16),
            pltpu.VMEM((3, (HB // 2) * (D + 8), DHB), U32),
            pltpu.VMEM((HB * DHB, D), BF16),
            pltpu.VMEM((HB * DHB // 2, D), U32),
            pltpu.SemaphoreType.DMA((NQ + 9,)),
            pltpu.SemaphoreType.DMA((NQ,)),
        ] + [pltpu.VMEM((BK, BQ), F32) for _ in range(2 * (S // BK))],
        compiler_params=pltpu.CompilerParams(vmem_limit_bytes=110 * 2**20, flags=FLAGS),
    )(
        A_x.reshape(S, D), A_wqkv, A_wo, B_mem0.reshape(M, D), gate_w.reshape(1, D),
        B_Wq, B_Wk, B_Wv, B_Wo.reshape(HB * DHB, D),
    )
    return out.reshape(Bn, S, D)
```

```python
import functools

import jax
import jax.numpy as jnp
import jax.experimental.pallas as pl
import jax.experimental.pallas.tpu as pltpu

G = 2
LAGS = (1, 2, 4)
BK = 128
BQ = 512
N0 = 4
MR = 128
UNR = 2


def APLAN(npos, n):
    return [[] for _ in range(npos - 4)] + [[0, 1], [2, 3], list(range(4, 16)), list(range(16, 32))]


SKIP = ()
NEWTON = True
WPAD = 1
QP = 128
VDENSE = True
QDENSE = True
FILLK = True
GAP = 0
PACEW = True
GDEP = True
GATE = 'vpu'
XB = 0
PACE = True
FLAGS = None
LOG2E = 1.4426950408889634
F32 = jnp.float32
BF16 = jnp.bfloat16
U32 = jnp.uint32
NN = (((1,), (0,)), ((), ()))
NT = (((1,), (1,)), ((), ()))
TN = (((0,), (0,)), ((), ()))


def _pk(x):
    return pltpu.bitcast(x.astype(BF16), U32)


def _unpk(x):
    return pltpu.bitcast(x, BF16)


def _dot(a, b, dims=NN):
    return jax.lax.dot_general(a, b, dims, preferred_element_type=F32)


def _interleave(main, side):
    n, k = len(main) - GAP, len(side)
    tok = None
    for i, f in enumerate(main):
        if i >= GAP:
            for g in side[(k * (i - GAP)) // n:(k * (i - GAP + 1)) // n]:
                g(tok)
        tok = f()


def _zero_after(tok):
    if tok is None or not PACE:
        return jnp.zeros((8, 128), U32)
    return pltpu.bitcast(jnp.abs(tok), U32) >> 31


def _make_kernel(S, D, HA, HB, DHB, M, SEG):
    DHA = D // HA
    NSEG = S // SEG
    L = M + SEG
    NQ = S // BQ
    NK = S // BK
    NU = HA * NQ
    GH = 128 // DHA
    VR = DHA + 8
    NG = HB // G
    SPQ = NSEG // NQ
    assert 2 * SPQ == HA and N0 % 2 == 0 and N0 >= 4
    WP = D + WPAD
    RL = 16
    PR = 128
    RQ = QP

    def kernel(x_hbm, wqkv_hbm, woa_hbm, mem0_ref, gw_ref,
               wq3_hbm, wk3_hbm, wv3_hbm, wob_hbm,
               out_hbm,
               x_ref, wqkv_ref, woa_ref, woap_ref,
               ka_ref, qm_ref, vt_ref, ma_ref, mb_ref, ot_ref,
               b_ref, g_ref, o_ref,
               w3_ref, wqkvb_ref, wob_stage, wob_ref, isems, osems, *sbufs):
        sa_ref, sb_ref = sbufs[:NK], sbufs[NK:]

        def x_copy(i):
            rows = pl.ds(pl.multiple_of(i * BQ, BQ), BQ)
            return pltpu.make_async_copy(x_hbm.at[rows], x_ref.at[rows], isems.at[i])

        def w3_copy(t, src):
            return pltpu.make_async_copy(src, w3_ref.at[t], isems.at[NQ + t])

        cp_wa = [pltpu.make_async_copy(wqkv_hbm.at[:, t * D:(t + 1) * D], wqkv_ref.at[:, t * D:(t + 1) * D],
                                       isems.at[NQ + 6 + t]) for t in range(3)]
        cp_wob = pltpu.make_async_copy(wob_hbm, wob_stage, isems.at[NQ + 4])
        cp_woa = pltpu.make_async_copy(woa_hbm, woa_ref, isems.at[NQ + 5])
        cp_wa[1].start()
        x_copy(0).start()
        x_copy(1).start()
        cp_wa[0].start()
        x_copy(2).start()
        cp_wa[2].start()
        for i in range(3, NQ):
            x_copy(i).start()
        for t, src in enumerate((wq3_hbm, wk3_hbm, wv3_hbm)):
            w3_copy(t, src).start()
        cp_wob.start()
        cp_woa.start()

        gw = gw_ref[...].astype(F32).reshape(1, D)
        gwb = jnp.broadcast_to(gw.astype(BF16), (128, D))
        qscale = (DHA ** -0.5) * LOG2E

        def fill(h, tok):
            z = _zero_after(tok)
            if not QDENSE:
                qm_ref[pl.ds(pl.multiple_of(h * 64, 64), 64), :] = jnp.tile(z, (8, S // 128))
            if not VDENSE:
                one = pltpu.bitcast(z | jnp.uint32(0x3F800000), F32)
                vt_ref[pl.ds(pl.multiple_of(h * VR + DHA, 8), VR - DHA), :] = jnp.tile(one, ((VR - DHA) // 8, S // 128))

        def fill_pad(h, tok):
            z = _zero_after(tok)
            zz = jnp.tile(z, (8, S // 128))
            rr = jax.lax.broadcasted_iota(jnp.int32, (64, S), 0)
            base = pl.multiple_of(h * 64, 64)
            for k in range(8):
                @pl.when(k != h % GH)
                def _():
                    qm_ref[pl.ds(base + 8 * k, 8), :] = zz[0:8]
            one = pltpu.bitcast(z | jnp.uint32(0x3F800000), F32)
            vt_ref[pl.ds(pl.multiple_of(h * VR + DHA, 8), VR - DHA), :] = jnp.tile(one, ((VR - DHA) // 8, S // 128))

        def proj_k(i, _):
            x_copy(i).wait()
            gz = []

            def piece(j):
                def f():
                    rows = pl.ds(pl.multiple_of(i * BQ + j * PR, PR), PR)
                    xb = x_ref[rows, :]
                    if GDEP and gz:
                        xd = _unpk(pltpu.bitcast(xb, U32) | jnp.tile(gz[-1], (PR // 16, D // 128)))
                    else:
                        xd = xb
                    kk = _dot(xd, wqkv_ref[:, D:2 * D])
                    ka_ref[pl.ds(pl.multiple_of((i * BQ + j * PR) // 2, PR // 2), PR // 2), :] = _pk(kk)
                    if GATE == 'vpu':
                        z = jnp.sum(xb.astype(F32) * gw, axis=1, keepdims=True)
                        gv = jnp.broadcast_to(jax.nn.sigmoid(z), (PR, 128))
                        g_ref[rows, :] = gv
                        gz.append(_zero_after(jnp.max(gv.reshape(PR // 8, 8, 128), axis=0)))
                    else:
                        g_ref[rows, :] = jax.nn.sigmoid(_dot(xb, gwb, NT))
                    return kk[0:8, 0:128]
                return f
            hpb = HA // NQ
            _interleave([piece(j) for j in range(BQ // PR)],
                        [functools.partial(fill, i * hpb + hh) for hh in range(hpb)] if FILLK else [])
            return 0
        if QDENSE:
            qm_ref[HA * 8:HA * 8 + 8, :] = jnp.zeros((8, S), U32)
        cp_wa[1].wait()
        jax.lax.fori_loop(0, NQ, proj_k, 0)

        cp_wa[0].wait()
        cp_wa[2].wait()
        wq_t = wqkv_ref[:, 0:D].astype(F32).T
        wv_t = wqkv_ref[:, 2 * D:3 * D].astype(F32).T

        def relayout(t, r, tok):
            z = _zero_after(tok)
            z = jnp.concatenate([z] * (HB // 16), axis=0)
            lo, hi = z | jnp.uint32(0xFFFF), z | jnp.uint32(0xFFFF0000)
            for j in range(r * RL // 2, (r + 1) * RL // 2):
                a = pltpu.bitcast(w3_ref[t, 2 * j], U32)
                b = pltpu.bitcast(w3_ref[t, 2 * j + 1], U32)
                e = (a & lo) | (b << 16)
                o = (a >> 16) | (b & hi)
                for i in range(HB // 16):
                    wqkvb_ref[t, pl.ds(8 * i * WP + j, 8, stride=WP), :] = e[8 * i:8 * i + 8]
                    wqkvb_ref[t, pl.ds(8 * i * WP + D // 2 + j, 8, stride=WP), :] = o[8 * i:8 * i + 8]

        def pack_wob(r, tok):
            w = _pk(wob_stage[r * 128:(r + 1) * 128, :])
            if PACEW:
                w = w | jnp.tile(_zero_after(tok), (8, D // 128))
            wob_ref[r * 64:(r + 1) * 64, :] = w

        def wslab(t, h):
            base = (h // 2) * WP + (h % 2) * (D // 2)
            return wqkvb_ref[t, base:base + D // 2, :]

        def proj_qv(i, _, side=False):
            cols = pl.ds(pl.multiple_of(i * BQ, BQ), BQ)

            def q_piece(j):
                def f():
                    qf = _dot(wq_t[j * RQ:(j + 1) * RQ], x_ref[cols, :], NT)
                    qt = _pk(qf * qscale)
                    for hh in range(RQ // DHA):
                        h = j * (RQ // DHA) + hh
                        r0 = h * 8 if QDENSE else (h * 128 + (h % GH) * DHA) // 2
                        qm_ref[r0:r0 + DHA // 2, cols] = qt[hh * DHA // 2:(hh + 1) * DHA // 2]
                    return qf[0:8, 0:128]
                return f

            def v_piece(j):
                def f():
                    vt = _dot(wv_t[j * RQ:(j + 1) * RQ], x_ref[cols, :], NT)
                    for hh in range(RQ // DHA):
                        h = j * (RQ // DHA) + hh
                        rq = h * (DHA if VDENSE else VR)
                        vt_ref[rq:rq + DHA, cols] = vt[hh * DHA:(hh + 1) * DHA]
                    return vt[0:8, 0:128]
                return f
            main = [f(j) for j in range(D // RQ) for f in (q_piece, v_piece)]
            if side:
                t = i - (NQ - 2)
                w3_copy(t, w3_ref.at[t]).wait()
                _interleave(main, [functools.partial(relayout, t, r) for r in range(D // RL)])
            elif FILLK:
                _interleave(main, [])
            else:
                hpb = HA // (NQ - 2)
                _interleave(main, [functools.partial(fill_pad, i * hpb + hh) for hh in range(hpb)])
            return 0
        jax.lax.fori_loop(0, NQ - 2, proj_qv, 0)
        jax.lax.fori_loop(NQ - 2, NQ, functools.partial(proj_qv, side=True), 0)

        def qcols(u):
            return pl.ds(pl.multiple_of((u // HA) * BQ, BQ), BQ)

        def s_chunk(u, c, buf):
            h = u % HA
            if QDENSE:
                qm = _unpk(jnp.concatenate([
                    qm_ref[pl.ds(pl.multiple_of(jnp.where(h % GH == k, h, HA) * 8, 8), 8), qcols(u)]
                    for k in range(GH)], axis=0))
            else:
                qm = _unpk(qm_ref[pl.ds(pl.multiple_of(h * 64, 64), 64), qcols(u)])
            kk = _unpk(ka_ref[c * BK // 2:(c + 1) * BK // 2, pl.ds(pl.multiple_of((h // GH) * 128, 128), 128)])
            st = _dot(kk, qm)
            buf[c][...] = st
            return jnp.max(st.reshape(BK // 8, 8, BQ), axis=0)

        def phase_tasks(u_s, buf_s, m_s, u_p, buf_p, m_p):
            st = {}
            hp = u_p % HA
            r0 = pl.multiple_of(hp * VR, 8)
            rv = pl.multiple_of(hp * DHA, DHA)

            def chunk(c):
                def f():
                    if c == 0:
                        st['m'] = m_p[...]
                        st['ot'] = jnp.zeros((VR, BQ), F32)
                        st['mx8'] = None
                    mc = s_chunk(u_s, c, buf_s)
                    st['mx8'] = mc if st['mx8'] is None else jnp.maximum(st['mx8'], mc)
                    p = jnp.exp2(buf_p[c][...] - st['m'])
                    if VDENSE:
                        vt = jnp.concatenate([vt_ref[pl.ds(rv, DHA), c * BK:(c + 1) * BK],
                                              jnp.ones((VR - DHA, BK), F32)], axis=0)
                    else:
                        vt = vt_ref[pl.ds(r0, VR), c * BK:(c + 1) * BK]
                    st['ot'] = st['ot'] + _dot(vt, p)
                    if c == NK - 1:
                        m_s[...] = jnp.max(st['mx8'], axis=0, keepdims=True)
                        ot = st['ot']
                        ot_ref[pl.ds(pl.multiple_of(hp * (DHA // 2), DHA // 2), DHA // 2), qcols(u_p)] = _pk(
                            ot[:DHA] / ot[DHA:DHA + 1])
                    return mc[:, 0:128]
                return f
            return [chunk(c) for c in range(NK)]

        def pair_tasks(u0):
            u1 = u0 + 1
            u2 = jnp.minimum(u0 + 2, NU - 1)
            return (phase_tasks(u1, sb_ref, mb_ref, u0, sa_ref, ma_ref)
                    + phase_tasks(u2, sa_ref, ma_ref, u1, sb_ref, mb_ref))

        first = {'mx8': None}

        def first_chunk(c):
            def f():
                mc = s_chunk(0, c, sa_ref)
                first['mx8'] = mc if first['mx8'] is None else jnp.maximum(first['mx8'], mc)
                return mc[:, 0:128]
            return f
        _interleave([first_chunk(c) for c in range(NK)], [])
        ma_ref[...] = jnp.max(first['mx8'], axis=0, keepdims=True)

        w3_copy(2, wv3_hbm).wait()
        _interleave(pair_tasks(0), [functools.partial(relayout, 2, r) for r in range(D // RL)])
        for j in range(1, N0 // 2):
            tasks = pair_tasks(2 * j)
            if j == N0 // 2 - 1:
                _interleave(tasks[:NK], [])
                cp_wob.wait()
                _interleave(tasks[NK:], [functools.partial(pack_wob, r) for r in range(HB * DHB // 128)])
            else:
                _interleave(tasks, [])
        cp_woa.wait()
        woap_ref[...] = _pk(woa_ref[...])

        row = jax.lax.broadcasted_iota(jnp.int32, (L, L), 0)
        col = jax.lax.broadcasted_iota(jnp.int32, (L, L), 1)
        allowed = (row >= SEG) | (col >= SEG) | (col <= row)
        bscale = (DHB ** -0.5) * LOG2E
        lS, lPV, lP = LAGS

        def step(s, mem, with_a=True):
            rows = pl.ds(pl.multiple_of(s * SEG, SEG), SEG)
            h = jnp.concatenate([x_ref[rows, :].astype(F32), mem], axis=0)

            def qkv(g):
                return tuple(
                    _dot(h, _unpk(jnp.concatenate([wslab(t, hh) for hh in range(g * G, (g + 1) * G)], axis=1)))
                    for t in range(3))

            def attn1(q, k, v):
                ps = []
                for j in range(G):
                    hs = slice(j * DHB, (j + 1) * DHB)
                    sc = _dot(q[:, hs], k[:, hs], NT) * bscale
                    sc = jnp.where(allowed, sc, -1e9 * LOG2E)
                    m = jnp.max(sc, axis=1, keepdims=True)
                    p = jnp.exp2(sc - m)
                    l = jnp.sum(p, axis=1, keepdims=True)
                    r = pl.reciprocal(l, approx=True)
                    if NEWTON:
                        r = r * (2.0 - l * r)
                    ps.append((p, r))
                return ps

            def attn2(ps, v):
                os_ = []
                for j in range(G):
                    hs = slice(j * DHB, (j + 1) * DHB)
                    p, rl = ps[j]
                    os_.append(_dot(p, v[:, hs]) * rl)
                return jnp.concatenate(os_, axis=1)

            acc = jnp.zeros((L, D), F32)
            QKV, PS, OG = {}, {}, {}
            if with_a:
                atasks = pair_tasks(2 * s + N0)
                plan = APLAN(NG + lP, len(atasks))
            else:
                plan = [[] for _ in range(NG + lP)]
            for g in range(NG + lP):
                for ti in plan[g]:
                    atasks[ti]()
                if g < NG:
                    QKV[g] = qkv(g)
                if 0 <= g - lS < NG:
                    PS[g - lS] = attn1(*QKV[g - lS])
                if 0 <= g - lPV < NG:
                    OG[g - lPV] = attn2(PS[g - lPV], QKV[g - lPV][2])
                if 0 <= g - lP < NG:
                    gg = g - lP
                    acc = acc + _dot(OG[gg], _unpk(wob_ref[gg * G * DHB // 2:(gg + 1) * G * DHB // 2, :]))
            b_ref[rows, :] = acc[:SEG]
            return acc[SEG:]

        def out_copy(q):
            rows = pl.ds(pl.multiple_of(q * BQ, BQ), BQ)
            return pltpu.make_async_copy(o_ref.at[rows], out_hbm.at[rows], osems.at[q])

        def mix(q):
            for j in range(BQ // MR):
                rows = pl.ds(pl.multiple_of(q * BQ + j * MR, MR), MR)
                a = _dot(_unpk(ot_ref[:, rows]), _unpk(woap_ref[...]), TN)
                g = g_ref[rows, :]
                g = jnp.concatenate([g] * (D // 128), axis=1)
                o_ref[rows, :] = (g * a + (1.0 - g) * b_ref[rows, :]).astype(o_ref.dtype)
            out_copy(q).start()

        NJ = NSEG - N0 // 2

        def steps(i, mem):
            for j in range(UNR):
                mem = step(i * UNR + j, mem)
            return mem

        def qblock(q, mem):
            if 'main' not in SKIP:
                mem = jax.lax.fori_loop(q * (SPQ // UNR), jnp.minimum((q + 1) * SPQ, NJ) // UNR, steps, mem)
            if 'mix' not in SKIP:
                pl.when(q < NQ - 1)(lambda: mix(q))
            return mem

        mem = jax.lax.fori_loop(0, NQ, qblock, mem0_ref[...].astype(F32))
        if 'bonly' not in SKIP:
            jax.lax.fori_loop(NJ - XB, NSEG, functools.partial(step, with_a=False), mem)
        if 'mix' not in SKIP:
            mix(NQ - 1)
            for q in range(NQ):
                out_copy(q).wait()

    return kernel


@functools.partial(jax.jit, static_argnames=("B_seg_len",))
def pallas_gated_mix__mha_block__memory_aug_recurrent_mem_tr__prompt_kernel(
    A_x, A_wqkv, A_wo, B_x, B_mem0, B_Wq, B_Wk, B_Wv, B_Wo, B_seg_len, gate_w,
):
    del B_x
    Bn, S, D = A_x.shape
    assert Bn == 1
    HA = 32
    _, HB, DHB = B_Wq.shape
    M = B_mem0.shape[1]
    SEG = int(B_seg_len)
    DHA = D // HA
    VR = DHA + 8
    NQ = S // BQ
    kernel = _make_kernel(S, D, HA, HB, DHB, M, SEG)
    vmem = pl.BlockSpec(memory_space=pltpu.VMEM)
    hbm = pl.BlockSpec(memory_space=pl.ANY)
    out = pl.pallas_call(
        kernel,
        out_shape=jax.ShapeDtypeStruct((S, D), A_x.dtype),
        in_specs=[hbm, hbm, hbm, vmem, vmem, hbm, hbm, hbm, hbm],
        out_specs=hbm,
        scratch_shapes=[
            pltpu.VMEM((S, D), BF16),
            pltpu.VMEM((D, 3 * D), BF16),
            pltpu.VMEM((D, D), BF16),
            pltpu.VMEM((D // 2, D), U32),
            pltpu.VMEM((S // 2, D), U32),
            pltpu.VMEM((HA * 8 + 8 if QDENSE else HA * 64, S), U32),
            pltpu.VMEM((HA * (DHA if VDENSE else VR), S), F32),
            pltpu.VMEM((1, BQ), F32),
            pltpu.VMEM((1, BQ), F32),
            pltpu.VMEM((D // 2, S), U32),
            pltpu.VMEM((S, D), F32),
            pltpu.VMEM((S, 128), F32),
            pltpu.VMEM((S, D), A_x.dtype),
            pltpu.VMEM((3, D, HB, DHB), BF16),
            pltpu.VMEM((3, -(-(HB // 2) * (D + WPAD) // 8) * 8, DHB), U32),
            pltpu.VMEM((HB * DHB, D), BF16),
            pltpu.VMEM((HB * DHB // 2, D), U32),
            pltpu.SemaphoreType.DMA((NQ + 9,)),
            pltpu.SemaphoreType.DMA((NQ,)),
        ] + [pltpu.VMEM((BK, BQ), F32) for _ in range(2 * (S // BK))],
        compiler_params=pltpu.CompilerParams(vmem_limit_bytes=110 * 2**20, flags=FLAGS),
    )(
        A_x.reshape(S, D), A_wqkv, A_wo, B_mem0.reshape(M, D), gate_w,
        B_Wq, B_Wk, B_Wv, B_Wo.reshape(HB * DHB, D),
    )
    return out.reshape(Bn, S, D)
```

```python
import functools

import jax
import jax.numpy as jnp
import jax.experimental.pallas as pl
import jax.experimental.pallas.tpu as pltpu

G = 2
LAGS = (1, 2, 4)
BK = 128
BQ = 512
N0 = 4
MR = 128
UNR = 2


def APLAN(npos, n):
    return [[] for _ in range(npos - 5)] + [[0], [1, 2, 3], list(range(4, 16)), [], list(range(16, 32))]


SKIP = ()
SUMK = 'sum'
MPULL = 0
ONES = False
PULL = 1
NEWTON = True
WPAD = 1
QP = 128
VDENSE = True
QDENSE = True
FILLK = True
GAP = 0
PACEW = True
GDEP = True
GATE = 'vpu'
XB = 0
PACE = True
FLAGS = None
LOG2E = 1.4426950408889634
F32 = jnp.float32
BF16 = jnp.bfloat16
U32 = jnp.uint32
NN = (((1,), (0,)), ((), ()))
NT = (((1,), (1,)), ((), ()))
TN = (((0,), (0,)), ((), ()))


def _pk(x):
    return pltpu.bitcast(x.astype(BF16), U32)


def _unpk(x):
    return pltpu.bitcast(x, BF16)


def _dot(a, b, dims=NN):
    return jax.lax.dot_general(a, b, dims, preferred_element_type=F32)


def _interleave(main, side):
    n, k = len(main) - GAP, len(side)
    tok = None
    for i, f in enumerate(main):
        if i >= GAP:
            for g in side[(k * (i - GAP)) // n:(k * (i - GAP + 1)) // n]:
                g(tok)
        tok = f()


def _zero_after(tok):
    if tok is None or not PACE:
        return jnp.zeros((8, 128), U32)
    return pltpu.bitcast(jnp.abs(tok), U32) >> 31


def _make_kernel(S, D, HA, HB, DHB, M, SEG):
    DHA = D // HA
    NSEG = S // SEG
    L = M + SEG
    NQ = S // BQ
    NK = S // BK
    NU = HA * NQ
    GH = 128 // DHA
    VR = DHA + 8
    NG = HB // G
    SPQ = NSEG // NQ
    assert 2 * SPQ == HA and N0 % 2 == 0 and N0 >= 4
    WP = D + WPAD
    RL = 16
    PR = 128
    RQ = QP

    def kernel(x_hbm, wqkv_hbm, woa_hbm, mem0_ref, gw_ref,
               wq3_hbm, wk3_hbm, wv3_hbm, wob_hbm,
               out_hbm,
               x_ref, wqkv_ref, woa_ref, woap_ref,
               ka_ref, qm_ref, vt_ref, ma_ref, mb_ref, ot_ref,
               b_ref, g_ref, o_ref,
               w3_ref, wqkvb_ref, wob_stage, wob_ref, isems, osems, *sbufs):
        sa_ref, sb_ref = sbufs[:NK], sbufs[NK:]

        def x_copy(i):
            rows = pl.ds(pl.multiple_of(i * BQ, BQ), BQ)
            return pltpu.make_async_copy(x_hbm.at[rows], x_ref.at[rows], isems.at[i])

        def w3_copy(t, src):
            return pltpu.make_async_copy(src, w3_ref.at[t], isems.at[NQ + t])

        cp_wa = [pltpu.make_async_copy(wqkv_hbm.at[:, t * D:(t + 1) * D], wqkv_ref.at[:, t * D:(t + 1) * D],
                                       isems.at[NQ + 6 + t]) for t in range(3)]
        cp_wob = pltpu.make_async_copy(wob_hbm, wob_stage, isems.at[NQ + 4])
        cp_woa = pltpu.make_async_copy(woa_hbm, woa_ref, isems.at[NQ + 5])
        cp_wa[1].start()
        x_copy(0).start()
        x_copy(1).start()
        cp_wa[0].start()
        x_copy(2).start()
        cp_wa[2].start()
        for i in range(3, NQ):
            x_copy(i).start()
        for t, src in enumerate((wq3_hbm, wk3_hbm, wv3_hbm)):
            w3_copy(t, src).start()
        cp_wob.start()
        cp_woa.start()

        gw = gw_ref[...].astype(F32).reshape(1, D)
        gwb = jnp.broadcast_to(gw.astype(BF16), (128, D))
        qscale = (DHA ** -0.5) * LOG2E

        def fill(h, tok):
            z = _zero_after(tok)
            if not QDENSE:
                qm_ref[pl.ds(pl.multiple_of(h * 64, 64), 64), :] = jnp.tile(z, (8, S // 128))
            if not VDENSE:
                one = pltpu.bitcast(z | jnp.uint32(0x3F800000), F32)
                vt_ref[pl.ds(pl.multiple_of(h * VR + DHA, 8), VR - DHA), :] = jnp.tile(one, ((VR - DHA) // 8, S // 128))

        def fill_pad(h, tok):
            z = _zero_after(tok)
            zz = jnp.tile(z, (8, S // 128))
            rr = jax.lax.broadcasted_iota(jnp.int32, (64, S), 0)
            base = pl.multiple_of(h * 64, 64)
            for k in range(8):
                @pl.when(k != h % GH)
                def _():
                    qm_ref[pl.ds(base + 8 * k, 8), :] = zz[0:8]
            one = pltpu.bitcast(z | jnp.uint32(0x3F800000), F32)
            vt_ref[pl.ds(pl.multiple_of(h * VR + DHA, 8), VR - DHA), :] = jnp.tile(one, ((VR - DHA) // 8, S // 128))

        def proj_k(i, _):
            x_copy(i).wait()
            gz = []

            def piece(j):
                def f():
                    rows = pl.ds(pl.multiple_of(i * BQ + j * PR, PR), PR)
                    xb = x_ref[rows, :]
                    if GDEP and gz:
                        xd = _unpk(pltpu.bitcast(xb, U32) | jnp.tile(gz[-1], (PR // 16, D // 128)))
                    else:
                        xd = xb
                    kk = _dot(xd, wqkv_ref[:, D:2 * D])
                    ka_ref[pl.ds(pl.multiple_of((i * BQ + j * PR) // 2, PR // 2), PR // 2), :] = _pk(kk)
                    if GATE == 'vpu':
                        z = jnp.sum(xb.astype(F32) * gw, axis=1, keepdims=True)
                        gv = jnp.broadcast_to(jax.nn.sigmoid(z), (PR, 128))
                        g_ref[rows, :] = gv
                        gz.append(_zero_after(jnp.max(gv.reshape(PR // 8, 8, 128), axis=0)))
                    else:
                        g_ref[rows, :] = jax.nn.sigmoid(_dot(xb, gwb, NT))
                    return kk[0:8, 0:128]
                return f
            hpb = HA // NQ
            _interleave([piece(j) for j in range(BQ // PR)],
                        [functools.partial(fill, i * hpb + hh) for hh in range(hpb)] if FILLK else [])
            return 0
        if QDENSE:
            qm_ref[HA * 8:HA * 8 + 8, :] = jnp.zeros((8, S), U32)
        cp_wa[1].wait()
        jax.lax.fori_loop(0, NQ, proj_k, 0)

        cp_wa[0].wait()
        cp_wa[2].wait()
        wq_t = wqkv_ref[:, 0:D].astype(F32).T
        wv_t = wqkv_ref[:, 2 * D:3 * D].astype(F32).T

        def relayout(t, r, tok):
            z = _zero_after(tok)
            z = jnp.concatenate([z] * (HB // 16), axis=0)
            lo, hi = z | jnp.uint32(0xFFFF), z | jnp.uint32(0xFFFF0000)
            for j in range(r * RL // 2, (r + 1) * RL // 2):
                a = pltpu.bitcast(w3_ref[t, 2 * j], U32)
                b = pltpu.bitcast(w3_ref[t, 2 * j + 1], U32)
                e = (a & lo) | (b << 16)
                o = (a >> 16) | (b & hi)
                for i in range(HB // 16):
                    wqkvb_ref[t, pl.ds(8 * i * WP + j, 8, stride=WP), :] = e[8 * i:8 * i + 8]
                    wqkvb_ref[t, pl.ds(8 * i * WP + D // 2 + j, 8, stride=WP), :] = o[8 * i:8 * i + 8]

        def pack_wob(r, tok):
            w = _pk(wob_stage[r * 128:(r + 1) * 128, :])
            if PACEW:
                w = w | jnp.tile(_zero_after(tok), (8, D // 128))
            wob_ref[r * 64:(r + 1) * 64, :] = w

        def wslab(t, h):
            base = (h // 2) * WP + (h % 2) * (D // 2)
            return wqkvb_ref[t, base:base + D // 2, :]

        def proj_qv(i, _, side=False):
            cols = pl.ds(pl.multiple_of(i * BQ, BQ), BQ)

            def q_piece(j):
                def f():
                    qf = _dot(wq_t[j * RQ:(j + 1) * RQ], x_ref[cols, :], NT)
                    qt = _pk(qf * qscale)
                    for hh in range(RQ // DHA):
                        h = j * (RQ // DHA) + hh
                        r0 = h * 8 if QDENSE else (h * 128 + (h % GH) * DHA) // 2
                        qm_ref[r0:r0 + DHA // 2, cols] = qt[hh * DHA // 2:(hh + 1) * DHA // 2]
                    return qf[0:8, 0:128]
                return f

            def v_piece(j):
                def f():
                    vt = _dot(wv_t[j * RQ:(j + 1) * RQ], x_ref[cols, :], NT)
                    for hh in range(RQ // DHA):
                        h = j * (RQ // DHA) + hh
                        rq = h * (DHA if VDENSE else VR)
                        vt_ref[rq:rq + DHA, cols] = vt[hh * DHA:(hh + 1) * DHA]
                    return vt[0:8, 0:128]
                return f
            main = [f(j) for j in range(D // RQ) for f in (q_piece, v_piece)]
            if side:
                t = i - (NQ - 2)
                w3_copy(t, w3_ref.at[t]).wait()
                _interleave(main, [functools.partial(relayout, t, r) for r in range(D // RL)])
            elif FILLK:
                _interleave(main, [])
            else:
                hpb = HA // (NQ - 2)
                _interleave(main, [functools.partial(fill_pad, i * hpb + hh) for hh in range(hpb)])
            return 0
        jax.lax.fori_loop(0, NQ - 2, proj_qv, 0)
        jax.lax.fori_loop(NQ - 2, NQ, functools.partial(proj_qv, side=True), 0)

        def qcols(u):
            return pl.ds(pl.multiple_of((u // HA) * BQ, BQ), BQ)

        def s_chunk(u, c, buf):
            h = u % HA
            if QDENSE:
                qm = _unpk(jnp.concatenate([
                    qm_ref[pl.ds(pl.multiple_of(jnp.where(h % GH == k, h, HA) * 8, 8), 8), qcols(u)]
                    for k in range(GH)], axis=0))
            else:
                qm = _unpk(qm_ref[pl.ds(pl.multiple_of(h * 64, 64), 64), qcols(u)])
            kk = _unpk(ka_ref[c * BK // 2:(c + 1) * BK // 2, pl.ds(pl.multiple_of((h // GH) * 128, 128), 128)])
            st = _dot(kk, qm)
            buf[c][...] = st
            return jnp.max(st.reshape(BK // 8, 8, BQ), axis=0)

        def phase_tasks(u_s, buf_s, m_s, u_p, buf_p, m_p):
            st = {}
            hp = u_p % HA
            r0 = pl.multiple_of(hp * VR, 8)
            rv = pl.multiple_of(hp * DHA, DHA)

            def chunk(c):
                def f():
                    if c == 0:
                        st['m'] = m_p[...]
                        st['ot'] = jnp.zeros((VR if ONES else DHA, BQ), F32)
                        st['mx8'] = None
                    mc = s_chunk(u_s, c, buf_s)
                    st['mx8'] = mc if st['mx8'] is None else jnp.maximum(st['mx8'], mc)
                    if c == 0:
                        st['l8'] = []
                        st['m8'] = jnp.broadcast_to(st['m'], (8, BQ))
                    if MPULL:
                        m8 = st['m8']
                        if c >= MPULL:
                            lz = st['l8'][c - MPULL]
                            z = jnp.concatenate([_zero_after(lz[:, jj * 128:(jj + 1) * 128]) for jj in range(BQ // 128)], axis=1)
                            m8 = pltpu.bitcast(pltpu.bitcast(m8, U32) | z, F32)
                        p = jnp.exp2(buf_p[c][...].reshape(BK // 8, 8, BQ) - m8[None]).reshape(BK, BQ)
                    else:
                        p = jnp.exp2(buf_p[c][...] - st['m'])
                    if not ONES:
                        vt = vt_ref[pl.ds(rv, DHA), c * BK:(c + 1) * BK]
                        if PULL and c >= PULL:
                            lz = st['l8'][c - PULL]
                            z = None
                            for jj in range(BQ // 128):
                                zz = _zero_after(lz[:, jj * 128:(jj + 1) * 128])
                                z = zz if z is None else z | zz
                            vt = pltpu.bitcast(pltpu.bitcast(vt, U32) | jnp.concatenate([z, z], axis=0), F32)
                        if SUMK == 'sum':
                            ls = jnp.sum(p.reshape(BK // 8, 8, BQ), axis=0)
                            st['l8'].append(ls if c == 0 else st['l8'][-1] + ls)
                        elif SUMK == 'tree':
                            parts = [p[8 * k:8 * k + 8] for k in range(BK // 8)]
                            while len(parts) > 1:
                                parts = [parts[2 * k] + parts[2 * k + 1] for k in range(len(parts) // 2)]
                            st['l8'].append(parts[0] if c == 0 else st['l8'][-1] + parts[0])
                        elif SUMK == 'chain':
                            acc8 = None if c == 0 else st['l8'][-1]
                            for k in range(BK // 8):
                                acc8 = p[8 * k:8 * k + 8] if acc8 is None else acc8 + p[8 * k:8 * k + 8]
                            st['l8'].append(acc8)
                        elif SUMK == 'chain2':
                            a0 = p[0:8]; a1 = p[8:16]
                            for k in range(2, BK // 8, 2):
                                a0 = a0 + p[8 * k:8 * k + 8]; a1 = a1 + p[8 * k + 8:8 * k + 16]
                            ls = a0 + a1
                            st['l8'].append(ls if c == 0 else st['l8'][-1] + ls)
                    elif VDENSE:
                        vt = jnp.concatenate([vt_ref[pl.ds(rv, DHA), c * BK:(c + 1) * BK],
                                              jnp.ones((VR - DHA, BK), F32)], axis=0)
                    else:
                        vt = vt_ref[pl.ds(r0, VR), c * BK:(c + 1) * BK]
                    st['ot'] = st['ot'] + _dot(vt, p)
                    if c == NK - 1:
                        m_s[...] = jnp.max(st['mx8'], axis=0, keepdims=True)
                        ot = st['ot']
                        l = ot[DHA:DHA + 1] if ONES else jnp.sum(st['l8'][-1], axis=0, keepdims=True)
                        ot_ref[pl.ds(pl.multiple_of(hp * (DHA // 2), DHA // 2), DHA // 2), qcols(u_p)] = _pk(
                            ot[:DHA] / l)
                    return mc[:, 0:128]
                return f
            return [chunk(c) for c in range(NK)]

        def pair_tasks(u0):
            u1 = u0 + 1
            u2 = jnp.minimum(u0 + 2, NU - 1)
            return (phase_tasks(u1, sb_ref, mb_ref, u0, sa_ref, ma_ref)
                    + phase_tasks(u2, sa_ref, ma_ref, u1, sb_ref, mb_ref))

        first = {'mx8': None}

        def first_chunk(c):
            def f():
                mc = s_chunk(0, c, sa_ref)
                first['mx8'] = mc if first['mx8'] is None else jnp.maximum(first['mx8'], mc)
                return mc[:, 0:128]
            return f
        _interleave([first_chunk(c) for c in range(NK)], [])
        ma_ref[...] = jnp.max(first['mx8'], axis=0, keepdims=True)

        w3_copy(2, wv3_hbm).wait()
        _interleave(pair_tasks(0), [functools.partial(relayout, 2, r) for r in range(D // RL)])
        for j in range(1, N0 // 2):
            tasks = pair_tasks(2 * j)
            if j == N0 // 2 - 1:
                _interleave(tasks[:NK], [])
                cp_wob.wait()
                _interleave(tasks[NK:], [functools.partial(pack_wob, r) for r in range(HB * DHB // 128)])
            else:
                _interleave(tasks, [])
        cp_woa.wait()
        woap_ref[...] = _pk(woa_ref[...])

        row = jax.lax.broadcasted_iota(jnp.int32, (L, L), 0)
        col = jax.lax.broadcasted_iota(jnp.int32, (L, L), 1)
        allowed = (row >= SEG) | (col >= SEG) | (col <= row)
        bscale = (DHB ** -0.5) * LOG2E
        lS, lPV, lP = LAGS

        def step(s, mem, with_a=True):
            rows = pl.ds(pl.multiple_of(s * SEG, SEG), SEG)
            h = jnp.concatenate([x_ref[rows, :].astype(F32), mem], axis=0)

            def qkv(g):
                return tuple(
                    _dot(h, _unpk(jnp.concatenate([wslab(t, hh) for hh in range(g * G, (g + 1) * G)], axis=1)))
                    for t in range(3))

            def attn1(q, k, v):
                ps = []
                for j in range(G):
                    hs = slice(j * DHB, (j + 1) * DHB)
                    sc = _dot(q[:, hs], k[:, hs], NT) * bscale
                    sc = jnp.where(allowed, sc, -1e9 * LOG2E)
                    m = jnp.max(sc, axis=1, keepdims=True)
                    p = jnp.exp2(sc - m)
                    l = jnp.sum(p, axis=1, keepdims=True)
                    r = pl.reciprocal(l, approx=True)
                    if NEWTON:
                        r = r * (2.0 - l * r)
                    ps.append((p, r))
                return ps

            def attn2(ps, v):
                os_ = []
                for j in range(G):
                    hs = slice(j * DHB, (j + 1) * DHB)
                    p, rl = ps[j]
                    os_.append(_dot(p, v[:, hs]) * rl)
                return jnp.concatenate(os_, axis=1)

            acc = jnp.zeros((L, D), F32)
            QKV, PS, OG = {}, {}, {}
            if with_a:
                atasks = pair_tasks(2 * s + N0)
                plan = APLAN(NG + lP, len(atasks))
            else:
                plan = [[] for _ in range(NG + lP)]
            for g in range(NG + lP):
                for ti in plan[g]:
                    atasks[ti]()
                if g < NG:
                    QKV[g] = qkv(g)
                if 0 <= g - lS < NG:
                    PS[g - lS] = attn1(*QKV[g - lS])
                if 0 <= g - lPV < NG:
                    OG[g - lPV] = attn2(PS[g - lPV], QKV[g - lPV][2])
                if 0 <= g - lP < NG:
                    gg = g - lP
                    acc = acc + _dot(OG[gg], _unpk(wob_ref[gg * G * DHB // 2:(gg + 1) * G * DHB // 2, :]))
            b_ref[rows, :] = acc[:SEG]
            return acc[SEG:]

        def out_copy(q):
            rows = pl.ds(pl.multiple_of(q * BQ, BQ), BQ)
            return pltpu.make_async_copy(o_ref.at[rows], out_hbm.at[rows], osems.at[q])

        def mix(q):
            for j in range(BQ // MR):
                rows = pl.ds(pl.multiple_of(q * BQ + j * MR, MR), MR)
                a = _dot(_unpk(ot_ref[:, rows]), _unpk(woap_ref[...]), TN)
                g = g_ref[rows, :]
                g = jnp.concatenate([g] * (D // 128), axis=1)
                o_ref[rows, :] = (g * a + (1.0 - g) * b_ref[rows, :]).astype(o_ref.dtype)
            out_copy(q).start()

        NJ = NSEG - N0 // 2

        def steps(i, mem):
            for j in range(UNR):
                mem = step(i * UNR + j, mem)
            return mem

        def qblock(q, mem):
            if 'main' not in SKIP:
                mem = jax.lax.fori_loop(q * (SPQ // UNR), jnp.minimum((q + 1) * SPQ, NJ) // UNR, steps, mem)
            if 'mix' not in SKIP:
                pl.when(q < NQ - 1)(lambda: mix(q))
            return mem

        mem = jax.lax.fori_loop(0, NQ, qblock, mem0_ref[...].astype(F32))
        if 'bonly' not in SKIP:
            jax.lax.fori_loop(NJ - XB, NSEG, functools.partial(step, with_a=False), mem)
        if 'mix' not in SKIP:
            mix(NQ - 1)
            for q in range(NQ):
                out_copy(q).wait()

    return kernel


@functools.partial(jax.jit, static_argnames=("B_seg_len",))
def pallas_gated_mix__mha_block__memory_aug_recurrent_mem_tr__prompt_kernel(
    A_x, A_wqkv, A_wo, B_x, B_mem0, B_Wq, B_Wk, B_Wv, B_Wo, B_seg_len, gate_w,
):
    del B_x
    Bn, S, D = A_x.shape
    assert Bn == 1
    HA = 32
    _, HB, DHB = B_Wq.shape
    M = B_mem0.shape[1]
    SEG = int(B_seg_len)
    DHA = D // HA
    VR = DHA + 8
    NQ = S // BQ
    kernel = _make_kernel(S, D, HA, HB, DHB, M, SEG)
    vmem = pl.BlockSpec(memory_space=pltpu.VMEM)
    hbm = pl.BlockSpec(memory_space=pl.ANY)
    out = pl.pallas_call(
        kernel,
        out_shape=jax.ShapeDtypeStruct((S, D), A_x.dtype),
        in_specs=[hbm, hbm, hbm, vmem, vmem, hbm, hbm, hbm, hbm],
        out_specs=hbm,
        scratch_shapes=[
            pltpu.VMEM((S, D), BF16),
            pltpu.VMEM((D, 3 * D), BF16),
            pltpu.VMEM((D, D), BF16),
            pltpu.VMEM((D // 2, D), U32),
            pltpu.VMEM((S // 2, D), U32),
            pltpu.VMEM((HA * 8 + 8 if QDENSE else HA * 64, S), U32),
            pltpu.VMEM((HA * (DHA if VDENSE else VR), S), F32),
            pltpu.VMEM((1, BQ), F32),
            pltpu.VMEM((1, BQ), F32),
            pltpu.VMEM((D // 2, S), U32),
            pltpu.VMEM((S, D), F32),
            pltpu.VMEM((S, 128), F32),
            pltpu.VMEM((S, D), A_x.dtype),
            pltpu.VMEM((3, D, HB, DHB), BF16),
            pltpu.VMEM((3, -(-(HB // 2) * (D + WPAD) // 8) * 8, DHB), U32),
            pltpu.VMEM((HB * DHB, D), BF16),
            pltpu.VMEM((HB * DHB // 2, D), U32),
            pltpu.SemaphoreType.DMA((NQ + 9,)),
            pltpu.SemaphoreType.DMA((NQ,)),
        ] + [pltpu.VMEM((BK, BQ), F32) for _ in range(2 * (S // BK))],
        compiler_params=pltpu.CompilerParams(vmem_limit_bytes=110 * 2**20, flags=FLAGS),
    )(
        A_x.reshape(S, D), A_wqkv, A_wo, B_mem0.reshape(M, D), gate_w,
        B_Wq, B_Wk, B_Wv, B_Wo.reshape(HB * DHB, D),
    )
    return out.reshape(Bn, S, D)
```

```python
import functools

import jax
import jax.numpy as jnp
import jax.experimental.pallas as pl
import jax.experimental.pallas.tpu as pltpu

G = 2
LAGS = (1, 2, 4)
BK = 128
BQ = 512
N0 = 4
UNR = 2
PR = 128
RL = 16

LOG2E = 1.4426950408889634
F32 = jnp.float32
BF16 = jnp.bfloat16
U32 = jnp.uint32
NN = (((1,), (0,)), ((), ()))
NT = (((1,), (1,)), ((), ()))
TN = (((0,), (0,)), ((), ()))


def APLAN(npos, n):
    counts = [0] * (npos - 5) + [1, 1, 14, 4, 12]
    assert sum(counts) == n
    starts = [sum(counts[:p]) for p in range(npos)]
    return [list(range(s, s + c)) for s, c in zip(starts, counts)]


def _pk(x):
    return pltpu.bitcast(x.astype(BF16), U32)


def _unpk(x):
    return pltpu.bitcast(x, BF16)


def _dot(a, b, dims=NN):
    return jax.lax.dot_general(a, b, dims, preferred_element_type=F32)


def _interleave(main, side):
    n, k = len(main), len(side)
    tok = None
    for i, f in enumerate(main):
        for g in side[(k * i) // n:(k * (i + 1)) // n]:
            g(tok)
        tok = f()


def _zero_after(tok):
    if tok is None:
        return jnp.zeros((8, 128), U32)
    return pltpu.bitcast(jnp.abs(tok), U32) >> 31


def _make_kernel(S, D, HA, HB, DHB, M, SEG):
    DHA = D // HA
    NSEG = S // SEG
    L = M + SEG
    NQ = S // BQ
    NK = S // BK
    NU = HA * NQ
    GH = 128 // DHA
    NG = HB // G
    SPQ = NSEG // NQ
    NJ = NSEG - N0 // 2
    WP = D + 1
    assert 2 * SPQ == HA and DHA == 16 and HB % 16 == 0 and NQ >= 3
    assert N0 % (2 * UNR) == 0 and N0 >= 4 and SPQ % UNR == 0

    def kernel(x_hbm, wqkv_hbm, woa_hbm, mem0_ref, gw_ref,
               wq3_hbm, wk3_hbm, wv3_hbm, wob_hbm,
               out_hbm,
               x_ref, wqkv_ref, woa_ref, woap_ref,
               ka_ref, qt_ref, vt_ref, ma_ref, mb_ref, ot_ref,
               b_ref, g_ref, o_ref,
               w3_ref, wqkvb_ref, wob_stage, wob_ref, isems, osems, *sbufs):
        sa_ref, sb_ref = sbufs[:NK], sbufs[NK:]

        def x_copy(i):
            rows = pl.ds(pl.multiple_of(i * BQ, BQ), BQ)
            return pltpu.make_async_copy(x_hbm.at[rows], x_ref.at[rows], isems.at[i])

        def w3_copy(t, src):
            return pltpu.make_async_copy(src, w3_ref.at[t], isems.at[NQ + t])

        cp_wob = pltpu.make_async_copy(wob_hbm, wob_stage, isems.at[NQ + 3])
        cp_woa = pltpu.make_async_copy(woa_hbm, woa_ref, isems.at[NQ + 4])
        cp_wa = [pltpu.make_async_copy(wqkv_hbm.at[:, t * D:(t + 1) * D], wqkv_ref.at[:, t * D:(t + 1) * D],
                                       isems.at[NQ + 5 + t]) for t in range(3)]
        cp_wa[1].start()
        x_copy(0).start()
        x_copy(1).start()
        cp_wa[0].start()
        x_copy(2).start()
        cp_wa[2].start()
        for i in range(3, NQ):
            x_copy(i).start()
        for t, src in enumerate((wq3_hbm, wk3_hbm, wv3_hbm)):
            w3_copy(t, src).start()
        cp_wob.start()
        cp_woa.start()

        gw = gw_ref[...].astype(F32).reshape(1, D)
        qscale = (DHA ** -0.5) * LOG2E
        qt_ref[HA * 8:HA * 8 + 8, :] = jnp.zeros((8, S), U32)

        def proj_k(i, _):
            x_copy(i).wait()
            gz = None
            for j in range(BQ // PR):
                rows = pl.ds(pl.multiple_of(i * BQ + j * PR, PR), PR)
                xb = x_ref[rows, :]
                xd = xb if gz is None else _unpk(pltpu.bitcast(xb, U32) | jnp.tile(gz, (PR // 16, D // 128)))
                ka_ref[pl.ds(pl.multiple_of((i * BQ + j * PR) // 2, PR // 2), PR // 2), :] = _pk(
                    _dot(xd, wqkv_ref[:, D:2 * D]))
                z = jnp.sum(xb.astype(F32) * gw, axis=1, keepdims=True)
                gv = jnp.broadcast_to(jax.nn.sigmoid(z), (PR, 128))
                g_ref[rows, :] = gv
                gz = _zero_after(jnp.max(gv.reshape(PR // 8, 8, 128), axis=0))
            return 0
        cp_wa[1].wait()
        jax.lax.fori_loop(0, NQ, proj_k, 0)

        def relayout(t, r, tok):
            z = jnp.concatenate([_zero_after(tok)] * (HB // 16), axis=0)
            lo, hi = z | jnp.uint32(0xFFFF), z | jnp.uint32(0xFFFF0000)
            for j in range(r * RL // 2, (r + 1) * RL // 2):
                a = pltpu.bitcast(w3_ref[t, 2 * j], U32)
                b = pltpu.bitcast(w3_ref[t, 2 * j + 1], U32)
                e = (a & lo) | (b << 16)
                o = (a >> 16) | (b & hi)
                for i in range(HB // 16):
                    wqkvb_ref[t, pl.ds(8 * i * WP + j, 8, stride=WP), :] = e[8 * i:8 * i + 8]
                    wqkvb_ref[t, pl.ds(8 * i * WP + D // 2 + j, 8, stride=WP), :] = o[8 * i:8 * i + 8]

        def relayout_tasks(t):
            return [functools.partial(relayout, t, r) for r in range(D // RL)]

        def pack_wob(r, tok):
            w = _pk(wob_stage[r * 128:(r + 1) * 128, :])
            wob_ref[r * 64:(r + 1) * 64, :] = w | jnp.tile(_zero_after(tok), (8, D // 128))

        def wslab(t, h):
            base = (h // 2) * WP + (h % 2) * (D // 2)
            return wqkvb_ref[t, base:base + D // 2, :]

        cp_wa[0].wait()
        cp_wa[2].wait()
        wq_t = wqkv_ref[:, 0:D].astype(F32).T
        wv_t = wqkv_ref[:, 2 * D:3 * D].astype(F32).T

        def proj_qv(i, _, side=False):
            cols = pl.ds(pl.multiple_of(i * BQ, BQ), BQ)

            def q_piece(j):
                def f():
                    qf = _dot(wq_t[j * PR:(j + 1) * PR], x_ref[cols, :], NT)
                    qt_ref[j * PR // 2:(j + 1) * PR // 2, cols] = _pk(qf * qscale)
                    return qf[0:8, 0:128]
                return f

            def v_piece(j):
                def f():
                    vt = _dot(wv_t[j * PR:(j + 1) * PR], x_ref[cols, :], NT)
                    vt_ref[j * PR:(j + 1) * PR, cols] = vt
                    return vt[0:8, 0:128]
                return f
            main = [f(j) for j in range(D // PR) for f in (q_piece, v_piece)]
            if side:
                t = i - (NQ - 2)
                w3_copy(t, w3_ref.at[t]).wait()
                _interleave(main, relayout_tasks(t))
            else:
                _interleave(main, [])
            return 0
        jax.lax.fori_loop(0, NQ - 2, proj_qv, 0)
        jax.lax.fori_loop(NQ - 2, NQ, functools.partial(proj_qv, side=True), 0)

        def qcols(u):
            return pl.ds(pl.multiple_of((u // HA) * BQ, BQ), BQ)

        def s_chunk(u, c, buf):
            h = u % HA
            qm = _unpk(jnp.concatenate([
                qt_ref[pl.ds(pl.multiple_of(jnp.where(h % GH == k, h, HA) * 8, 8), 8), qcols(u)]
                for k in range(GH)], axis=0))
            kk = _unpk(ka_ref[c * BK // 2:(c + 1) * BK // 2, pl.ds(pl.multiple_of((h // GH) * 128, 128), 128)])
            st = _dot(kk, qm)
            buf[c][...] = st
            return jnp.max(st.reshape(BK // 8, 8, BQ), axis=0)

        def phase_tasks(u_s, buf_s, m_s, u_p, buf_p, m_p):
            st = {}
            hp = u_p % HA
            rv = pl.multiple_of(hp * DHA, DHA)

            def chunk(c):
                def f():
                    keys = slice(c * BK, (c + 1) * BK)
                    if c == 0:
                        st['m'] = m_p[...]
                        st['ot'] = jnp.zeros((DHA, BQ), F32)
                        st['mx8'] = None
                    mc = s_chunk(u_s, c, buf_s)
                    st['mx8'] = mc if st['mx8'] is None else jnp.maximum(st['mx8'], mc)
                    p = jnp.exp2(buf_p[c][...] - st['m'])
                    vt = vt_ref[pl.ds(rv, DHA), keys]
                    if c > 0:
                        z = None
                        for jj in range(BQ // 128):
                            zz = _zero_after(st['l8'][:, jj * 128:(jj + 1) * 128])
                            z = zz if z is None else z | zz
                        vt = pltpu.bitcast(pltpu.bitcast(vt, U32) | jnp.concatenate([z, z], axis=0), F32)
                    ls = jnp.sum(p.reshape(BK // 8, 8, BQ), axis=0)
                    st['l8'] = ls if c == 0 else st['l8'] + ls
                    st['ot'] = st['ot'] + _dot(vt, p)
                    if c == NK - 1:
                        m_s[...] = jnp.max(st['mx8'], axis=0, keepdims=True)
                        l = jnp.sum(st['l8'], axis=0, keepdims=True)
                        ot_ref[pl.ds(pl.multiple_of(hp * (DHA // 2), DHA // 2), DHA // 2), qcols(u_p)] = _pk(
                            st['ot'] / l)
                    return mc[:, 0:128]
                return f
            return [chunk(c) for c in range(NK)]

        def pair_tasks(u0):
            u1 = u0 + 1
            u2 = jnp.minimum(u0 + 2, NU - 1)
            return (phase_tasks(u1, sb_ref, mb_ref, u0, sa_ref, ma_ref)
                    + phase_tasks(u2, sa_ref, ma_ref, u1, sb_ref, mb_ref))

        mx8 = None
        for c in range(NK):
            mc = s_chunk(0, c, sa_ref)
            mx8 = mc if mx8 is None else jnp.maximum(mx8, mc)
        ma_ref[...] = jnp.max(mx8, axis=0, keepdims=True)

        w3_copy(2, wv3_hbm).wait()
        _interleave(pair_tasks(0), relayout_tasks(2))
        for j in range(1, N0 // 2):
            tasks = pair_tasks(2 * j)
            if j == N0 // 2 - 1:
                _interleave(tasks[:NK], [])
                cp_wob.wait()
                _interleave(tasks[NK:], [functools.partial(pack_wob, r) for r in range(HB * DHB // 128)])
            else:
                _interleave(tasks, [])
        cp_woa.wait()
        woap_ref[...] = _pk(woa_ref[...])

        row = jax.lax.broadcasted_iota(jnp.int32, (L, L), 0)
        col = jax.lax.broadcasted_iota(jnp.int32, (L, L), 1)
        allowed = (row >= SEG) | (col >= SEG) | (col <= row)
        bscale = (DHB ** -0.5) * LOG2E
        lS, lPV, lP = LAGS

        def step(s, mem, with_a=True):
            rows = pl.ds(pl.multiple_of(s * SEG, SEG), SEG)
            h = jnp.concatenate([x_ref[rows, :].astype(F32), mem], axis=0)

            def qkv(g):
                return tuple(
                    _dot(h, _unpk(jnp.concatenate([wslab(t, hh) for hh in range(g * G, (g + 1) * G)], axis=1)))
                    for t in range(3))

            def probs(q, k, v):
                ps = []
                for j in range(G):
                    hs = slice(j * DHB, (j + 1) * DHB)
                    sc = _dot(q[:, hs], k[:, hs], NT) * bscale
                    sc = jnp.where(allowed, sc, -1e9 * LOG2E)
                    m = jnp.max(sc, axis=1, keepdims=True)
                    p = jnp.exp2(sc - m)
                    l = jnp.sum(p, axis=1, keepdims=True)
                    r = pl.reciprocal(l, approx=True)
                    ps.append((p, r * (2.0 - l * r)))
                return ps

            def values(ps, v):
                return jnp.concatenate(
                    [_dot(p, v[:, j * DHB:(j + 1) * DHB]) * rl for j, (p, rl) in enumerate(ps)], axis=1)

            acc = jnp.zeros((L, D), F32)
            QKV, PS, OG = {}, {}, {}
            if with_a:
                atasks = pair_tasks(2 * s + N0)
                plan = APLAN(NG + lP, len(atasks))
            else:
                plan = [[] for _ in range(NG + lP)]
            for g in range(NG + lP):
                for ti in plan[g]:
                    atasks[ti]()
                if g < NG:
                    QKV[g] = qkv(g)
                if 0 <= g - lS < NG:
                    PS[g - lS] = probs(*QKV[g - lS])
                if 0 <= g - lPV < NG:
                    OG[g - lPV] = values(PS[g - lPV], QKV[g - lPV][2])
                if 0 <= g - lP < NG:
                    wr = (g - lP) * G * DHB // 2
                    acc = acc + _dot(OG[g - lP], _unpk(wob_ref[wr:wr + G * DHB // 2, :]))
            b_ref[rows, :] = acc[:SEG]
            return acc[SEG:]

        def out_copy(q):
            rows = pl.ds(pl.multiple_of(q * BQ, BQ), BQ)
            return pltpu.make_async_copy(o_ref.at[rows], out_hbm.at[rows], osems.at[q])

        def mix(q):
            for j in range(BQ // PR):
                rows = pl.ds(pl.multiple_of(q * BQ + j * PR, PR), PR)
                a = _dot(_unpk(ot_ref[:, rows]), _unpk(woap_ref[...]), TN)
                g = g_ref[rows, :]
                g = jnp.concatenate([g] * (D // 128), axis=1)
                o_ref[rows, :] = (g * a + (1.0 - g) * b_ref[rows, :]).astype(o_ref.dtype)
            out_copy(q).start()

        def steps(i, mem):
            for j in range(UNR):
                mem = step(i * UNR + j, mem)
            return mem

        def qblock(q, mem):
            mem = jax.lax.fori_loop(q * (SPQ // UNR), jnp.minimum((q + 1) * SPQ, NJ) // UNR, steps, mem)
            pl.when(q < NQ - 1)(lambda: mix(q))
            return mem

        mem = jax.lax.fori_loop(0, NQ, qblock, mem0_ref[...].astype(F32))
        jax.lax.fori_loop(NJ, NSEG, functools.partial(step, with_a=False), mem)
        mix(NQ - 1)
        for q in range(NQ):
            out_copy(q).wait()

    return kernel


@functools.partial(jax.jit, static_argnames=("B_seg_len",))
def pallas_gated_mix__mha_block__memory_aug_recurrent_mem_tr__prompt_kernel(
    A_x, A_wqkv, A_wo, B_x, B_mem0, B_Wq, B_Wk, B_Wv, B_Wo, B_seg_len, gate_w,
):
    del B_x
    Bn, S, D = A_x.shape
    assert Bn == 1
    HA = 32
    _, HB, DHB = B_Wq.shape
    M = B_mem0.shape[1]
    SEG = int(B_seg_len)
    NQ = S // BQ
    kernel = _make_kernel(S, D, HA, HB, DHB, M, SEG)
    vmem = pl.BlockSpec(memory_space=pltpu.VMEM)
    hbm = pl.BlockSpec(memory_space=pl.ANY)
    out = pl.pallas_call(
        kernel,
        out_shape=jax.ShapeDtypeStruct((S, D), A_x.dtype),
        in_specs=[hbm, hbm, hbm, vmem, vmem, hbm, hbm, hbm, hbm],
        out_specs=hbm,
        scratch_shapes=[
            pltpu.VMEM((S, D), BF16),
            pltpu.VMEM((D, 3 * D), BF16),
            pltpu.VMEM((D, D), BF16),
            pltpu.VMEM((D // 2, D), U32),
            pltpu.VMEM((S // 2, D), U32),
            pltpu.VMEM((D // 2 + 8, S), U32),
            pltpu.VMEM((D, S), F32),
            pltpu.VMEM((1, BQ), F32),
            pltpu.VMEM((1, BQ), F32),
            pltpu.VMEM((D // 2, S), U32),
            pltpu.VMEM((S, D), F32),
            pltpu.VMEM((S, 128), F32),
            pltpu.VMEM((S, D), A_x.dtype),
            pltpu.VMEM((3, D, HB, DHB), BF16),
            pltpu.VMEM((3, -(-(HB // 2) * (D + 1) // 8) * 8, DHB), U32),
            pltpu.VMEM((HB * DHB, D), BF16),
            pltpu.VMEM((HB * DHB // 2, D), U32),
            pltpu.SemaphoreType.DMA((NQ + 8,)),
            pltpu.SemaphoreType.DMA((NQ,)),
        ] + [pltpu.VMEM((BK, BQ), F32) for _ in range(2 * (S // BK))],
        compiler_params=pltpu.CompilerParams(vmem_limit_bytes=110 * 2**20),
    )(
        A_x.reshape(S, D), A_wqkv, A_wo, B_mem0.reshape(M, D), gate_w,
        B_Wq, B_Wk, B_Wv, B_Wo.reshape(HB * DHB, D),
    )
    return out.reshape(Bn, S, D)
```

```python
import functools

import jax
import jax.numpy as jnp
import jax.experimental.pallas as pl
import jax.experimental.pallas.tpu as pltpu

G = 2
LAGS = (1, 2, 4)
BK = 128
BQ = 512
N0 = 4
UNR = 2
PR = 128
RL = 16

LOG2E = 1.4426950408889634
F32 = jnp.float32
BF16 = jnp.bfloat16
U32 = jnp.uint32
NN = (((1,), (0,)), ((), ()))
NT = (((1,), (1,)), ((), ()))
TN = (((0,), (0,)), ((), ()))
TT = (((0,), (1,)), ((), ()))


def APLAN(npos, n):
    counts = [0] * (npos - 5) + [1, 1, 14, 4, 12]
    assert sum(counts) == n
    starts = [sum(counts[:p]) for p in range(npos)]
    return [list(range(s, s + c)) for s, c in zip(starts, counts)]


def _pk(x):
    return pltpu.bitcast(x.astype(BF16), U32)


def _unpk(x):
    return pltpu.bitcast(x, BF16)


def _dot(a, b, dims=NN):
    return jax.lax.dot_general(a, b, dims, preferred_element_type=F32)


def _interleave(main, side):
    n, k = len(main), len(side)
    tok = None
    for i, f in enumerate(main):
        for g in side[(k * i) // n:(k * (i + 1)) // n]:
            g(tok)
        tok = f()


def _zero_after(tok):
    if tok is None:
        return jnp.zeros((8, 128), U32)
    return pltpu.bitcast(jnp.abs(tok), U32) >> 31


def _make_kernel(S, D, HA, HB, DHB, M, SEG):
    DHA = D // HA
    NSEG = S // SEG
    L = M + SEG
    NQ = S // BQ
    NK = S // BK
    NU = HA * NQ
    GH = 128 // DHA
    NG = HB // G
    SPQ = NSEG // NQ
    NJ = NSEG - N0 // 2
    WP = D + 1
    assert 2 * SPQ == HA and DHA == 16 and HB % 16 == 0 and NQ >= 3
    assert N0 % (2 * UNR) == 0 and N0 >= 4 and SPQ % UNR == 0

    def kernel(x_hbm, wqkv_hbm, woa_hbm, mem0_ref, gw_ref,
               wq3_hbm, wk3_hbm, wv3_hbm, wob_hbm,
               out_hbm,
               x_ref, wqkv_ref, woa_ref, woap_ref,
               ka_ref, qt_ref, vt_ref, ma_ref, mb_ref, ot_ref,
               b_ref, g_ref, o_ref,
               w3_ref, wqkvb_ref, wob_stage, wob_ref, isems, osems, *sbufs):
        sa_ref, sb_ref = sbufs[:NK], sbufs[NK:]

        def x_copy(i):
            rows = pl.ds(pl.multiple_of(i * BQ, BQ), BQ)
            return pltpu.make_async_copy(x_hbm.at[rows], x_ref.at[rows], isems.at[i])

        def w3_copy(t, src):
            return pltpu.make_async_copy(src, w3_ref.at[t], isems.at[NQ + t])

        cp_wob = pltpu.make_async_copy(wob_hbm, wob_stage, isems.at[NQ + 3])
        cp_woa = pltpu.make_async_copy(woa_hbm, woa_ref, isems.at[NQ + 4])
        cp_wa = [pltpu.make_async_copy(wqkv_hbm.at[:, t * D:(t + 1) * D], wqkv_ref.at[:, t * D:(t + 1) * D],
                                       isems.at[NQ + 5 + t]) for t in range(3)]
        cp_wa[1].start()
        x_copy(0).start()
        x_copy(1).start()
        cp_wa[0].start()
        x_copy(2).start()
        cp_wa[2].start()
        for i in range(3, NQ):
            x_copy(i).start()
        for t, src in enumerate((wq3_hbm, wk3_hbm, wv3_hbm)):
            w3_copy(t, src).start()
        cp_wob.start()
        cp_woa.start()

        gw = gw_ref[...].astype(F32).reshape(1, D)
        qscale = (DHA ** -0.5) * LOG2E
        qt_ref[HA * 8:HA * 8 + 8, :] = jnp.zeros((8, S), U32)

        def proj_k(i, _):
            x_copy(i).wait()
            gz = None
            for j in range(BQ // PR):
                rows = pl.ds(pl.multiple_of(i * BQ + j * PR, PR), PR)
                xb = x_ref[rows, :]
                xd = xb if gz is None else _unpk(pltpu.bitcast(xb, U32) | jnp.tile(gz, (PR // 16, D // 128)))
                ka_ref[pl.ds(pl.multiple_of((i * BQ + j * PR) // 2, PR // 2), PR // 2), :] = _pk(
                    _dot(xd, wqkv_ref[:, D:2 * D]))
                z = jnp.sum(xb.astype(F32) * gw, axis=1, keepdims=True)
                gv = jnp.broadcast_to(jax.nn.sigmoid(z), (PR, 128))
                g_ref[rows, :] = gv
                gz = _zero_after(jnp.max(gv.reshape(PR // 8, 8, 128), axis=0))
            return 0
        cp_wa[1].wait()
        jax.lax.fori_loop(0, NQ, proj_k, 0)

        def relayout(t, r, tok):
            z = jnp.concatenate([_zero_after(tok)] * (HB // 16), axis=0)
            lo, hi = z | jnp.uint32(0xFFFF), z | jnp.uint32(0xFFFF0000)
            for j in range(r * RL // 2, (r + 1) * RL // 2):
                a = pltpu.bitcast(w3_ref[t, 2 * j], U32)
                b = pltpu.bitcast(w3_ref[t, 2 * j + 1], U32)
                e = (a & lo) | (b << 16)
                o = (a >> 16) | (b & hi)
                for i in range(HB // 16):
                    wqkvb_ref[t, pl.ds(8 * i * WP + j, 8, stride=WP), :] = e[8 * i:8 * i + 8]
                    wqkvb_ref[t, pl.ds(8 * i * WP + D // 2 + j, 8, stride=WP), :] = o[8 * i:8 * i + 8]

        def relayout_tasks(t):
            return [functools.partial(relayout, t, r) for r in range(D // RL)]

        def pack_wob(r, tok):
            w = _pk(wob_stage[r * 128:(r + 1) * 128, :])
            wob_ref[r * 64:(r + 1) * 64, :] = w | jnp.tile(_zero_after(tok), (8, D // 128))

        def wslab(t, h):
            base = (h // 2) * WP + (h % 2) * (D // 2)
            return wqkvb_ref[t, base:base + D // 2, :]

        cp_wa[0].wait()
        cp_wa[2].wait()

        def proj_qv(i, _, side=False):
            cols = pl.ds(pl.multiple_of(i * BQ, BQ), BQ)

            def q_piece(j):
                def f():
                    qf = _dot(wqkv_ref[:, j * PR:(j + 1) * PR], x_ref[cols, :], TT)
                    qt_ref[j * PR // 2:(j + 1) * PR // 2, cols] = _pk(qf * qscale)
                    return qf[0:8, 0:128]
                return f

            def v_piece(j):
                def f():
                    vt = _dot(wqkv_ref[:, 2 * D + j * PR:2 * D + (j + 1) * PR], x_ref[cols, :], TT)
                    vt_ref[j * PR:(j + 1) * PR, cols] = vt
                    return vt[0:8, 0:128]
                return f
            main = [f(j) for j in range(D // PR) for f in (q_piece, v_piece)]
            if side:
                t = i - (NQ - 2)
                w3_copy(t, w3_ref.at[t]).wait()
                _interleave(main, relayout_tasks(t))
            else:
                _interleave(main, [])
            return 0
        jax.lax.fori_loop(0, NQ - 2, proj_qv, 0)
        jax.lax.fori_loop(NQ - 2, NQ, functools.partial(proj_qv, side=True), 0)

        def qcols(u):
            return pl.ds(pl.multiple_of((u // HA) * BQ, BQ), BQ)

        def s_chunk(u, c, buf):
            h = u % HA
            qm = _unpk(jnp.concatenate([
                qt_ref[pl.ds(pl.multiple_of(jnp.where(h % GH == k, h, HA) * 8, 8), 8), qcols(u)]
                for k in range(GH)], axis=0))
            kk = _unpk(ka_ref[c * BK // 2:(c + 1) * BK // 2, pl.ds(pl.multiple_of((h // GH) * 128, 128), 128)])
            st = _dot(kk, qm)
            buf[c][...] = st
            return jnp.max(st.reshape(BK // 8, 8, BQ), axis=0)

        def phase_tasks(u_s, buf_s, m_s, u_p, buf_p, m_p):
            st = {}
            hp = u_p % HA
            rv = pl.multiple_of(hp * DHA, DHA)

            def chunk(c):
                def f():
                    keys = slice(c * BK, (c + 1) * BK)
                    if c == 0:
                        st['m'] = m_p[...]
                        st['ot'] = jnp.zeros((DHA, BQ), F32)
                        st['mx8'] = None
                    mc = s_chunk(u_s, c, buf_s)
                    st['mx8'] = mc if st['mx8'] is None else jnp.maximum(st['mx8'], mc)
                    p = jnp.exp2(buf_p[c][...] - st['m'])
                    vt = vt_ref[pl.ds(rv, DHA), keys]
                    if c > 0:
                        z = None
                        for jj in range(BQ // 128):
                            zz = _zero_after(st['l8'][:, jj * 128:(jj + 1) * 128])
                            z = zz if z is None else z | zz
                        vt = pltpu.bitcast(pltpu.bitcast(vt, U32) | jnp.concatenate([z, z], axis=0), F32)
                    ls = jnp.sum(p.reshape(BK // 8, 8, BQ), axis=0)
                    st['l8'] = ls if c == 0 else st['l8'] + ls
                    st['ot'] = st['ot'] + _dot(vt, p)
                    if c == NK - 1:
                        m_s[...] = jnp.max(st['mx8'], axis=0, keepdims=True)
                        l = jnp.sum(st['l8'], axis=0, keepdims=True)
                        ot_ref[pl.ds(pl.multiple_of(hp * (DHA // 2), DHA // 2), DHA // 2), qcols(u_p)] = _pk(
                            st['ot'] / l)
                    return mc[:, 0:128]
                return f
            return [chunk(c) for c in range(NK)]

        def pair_tasks(u0):
            u1 = u0 + 1
            u2 = jnp.minimum(u0 + 2, NU - 1)
            return (phase_tasks(u1, sb_ref, mb_ref, u0, sa_ref, ma_ref)
                    + phase_tasks(u2, sa_ref, ma_ref, u1, sb_ref, mb_ref))

        mx8 = None
        for c in range(NK):
            mc = s_chunk(0, c, sa_ref)
            mx8 = mc if mx8 is None else jnp.maximum(mx8, mc)
        ma_ref[...] = jnp.max(mx8, axis=0, keepdims=True)

        w3_copy(2, wv3_hbm).wait()
        _interleave(pair_tasks(0), relayout_tasks(2))
        for j in range(1, N0 // 2):
            tasks = pair_tasks(2 * j)
            if j == N0 // 2 - 1:
                _interleave(tasks[:NK], [])
                cp_wob.wait()
                _interleave(tasks[NK:], [functools.partial(pack_wob, r) for r in range(HB * DHB // 128)])
            else:
                _interleave(tasks, [])
        cp_woa.wait()
        woap_ref[...] = _pk(woa_ref[...])

        row = jax.lax.broadcasted_iota(jnp.int32, (L, L), 0)
        col = jax.lax.broadcasted_iota(jnp.int32, (L, L), 1)
        allowed = (row >= SEG) | (col >= SEG) | (col <= row)
        bscale = (DHB ** -0.5) * LOG2E
        lS, lPV, lP = LAGS

        def step(s, mem, with_a=True):
            rows = pl.ds(pl.multiple_of(s * SEG, SEG), SEG)
            h = jnp.concatenate([x_ref[rows, :].astype(F32), mem], axis=0)

            def qkv(g):
                return tuple(
                    _dot(h, _unpk(jnp.concatenate([wslab(t, hh) for hh in range(g * G, (g + 1) * G)], axis=1)))
                    for t in range(3))

            def probs(q, k, v):
                ps = []
                for j in range(G):
                    hs = slice(j * DHB, (j + 1) * DHB)
                    sc = _dot(q[:, hs], k[:, hs], NT) * bscale
                    sc = jnp.where(allowed, sc, -1e9 * LOG2E)
                    m = jnp.max(sc, axis=1, keepdims=True)
                    p = jnp.exp2(sc - m)
                    l = jnp.sum(p, axis=1, keepdims=True)
                    r = pl.reciprocal(l, approx=True)
                    ps.append((p, r * (2.0 - l * r)))
                return ps

            def values(ps, v):
                return jnp.concatenate(
                    [_dot(p, v[:, j * DHB:(j + 1) * DHB]) * rl for j, (p, rl) in enumerate(ps)], axis=1)

            acc = jnp.zeros((L, D), F32)
            QKV, PS, OG = {}, {}, {}
            if with_a:
                atasks = pair_tasks(2 * s + N0)
                plan = APLAN(NG + lP, len(atasks))
            else:
                plan = [[] for _ in range(NG + lP)]
            for g in range(NG + lP):
                for ti in plan[g]:
                    atasks[ti]()
                if g < NG:
                    QKV[g] = qkv(g)
                if 0 <= g - lS < NG:
                    PS[g - lS] = probs(*QKV[g - lS])
                if 0 <= g - lPV < NG:
                    OG[g - lPV] = values(PS[g - lPV], QKV[g - lPV][2])
                if 0 <= g - lP < NG:
                    wr = (g - lP) * G * DHB // 2
                    acc = acc + _dot(OG[g - lP], _unpk(wob_ref[wr:wr + G * DHB // 2, :]))
            b_ref[rows, :] = acc[:SEG]
            return acc[SEG:]

        def out_copy(q):
            rows = pl.ds(pl.multiple_of(q * BQ, BQ), BQ)
            return pltpu.make_async_copy(o_ref.at[rows], out_hbm.at[rows], osems.at[q])

        def mix(q):
            for j in range(BQ // PR):
                rows = pl.ds(pl.multiple_of(q * BQ + j * PR, PR), PR)
                a = _dot(_unpk(ot_ref[:, rows]), _unpk(woap_ref[...]), TN)
                g = g_ref[rows, :]
                g = jnp.concatenate([g] * (D // 128), axis=1)
                o_ref[rows, :] = (g * a + (1.0 - g) * b_ref[rows, :]).astype(o_ref.dtype)
            out_copy(q).start()

        def steps(i, mem):
            for j in range(UNR):
                mem = step(i * UNR + j, mem)
            return mem

        def qblock(q, mem):
            mem = jax.lax.fori_loop(q * (SPQ // UNR), jnp.minimum((q + 1) * SPQ, NJ) // UNR, steps, mem)
            pl.when(q < NQ - 1)(lambda: mix(q))
            return mem

        mem = jax.lax.fori_loop(0, NQ, qblock, mem0_ref[...].astype(F32))
        jax.lax.fori_loop(NJ, NSEG, functools.partial(step, with_a=False), mem)
        mix(NQ - 1)
        for q in range(NQ):
            out_copy(q).wait()

    return kernel


@functools.partial(jax.jit, static_argnames=("B_seg_len",))
def pallas_gated_mix__mha_block__memory_aug_recurrent_mem_tr__prompt_kernel(
    A_x, A_wqkv, A_wo, B_x, B_mem0, B_Wq, B_Wk, B_Wv, B_Wo, B_seg_len, gate_w,
):
    del B_x
    Bn, S, D = A_x.shape
    assert Bn == 1
    HA = 32
    _, HB, DHB = B_Wq.shape
    M = B_mem0.shape[1]
    SEG = int(B_seg_len)
    NQ = S // BQ
    kernel = _make_kernel(S, D, HA, HB, DHB, M, SEG)
    vmem = pl.BlockSpec(memory_space=pltpu.VMEM)
    hbm = pl.BlockSpec(memory_space=pl.ANY)
    out = pl.pallas_call(
        kernel,
        out_shape=jax.ShapeDtypeStruct((S, D), A_x.dtype),
        in_specs=[hbm, hbm, hbm, vmem, vmem, hbm, hbm, hbm, hbm],
        out_specs=hbm,
        scratch_shapes=[
            pltpu.VMEM((S, D), BF16),
            pltpu.VMEM((D, 3 * D), BF16),
            pltpu.VMEM((D, D), BF16),
            pltpu.VMEM((D // 2, D), U32),
            pltpu.VMEM((S // 2, D), U32),
            pltpu.VMEM((D // 2 + 8, S), U32),
            pltpu.VMEM((D, S), F32),
            pltpu.VMEM((1, BQ), F32),
            pltpu.VMEM((1, BQ), F32),
            pltpu.VMEM((D // 2, S), U32),
            pltpu.VMEM((S, D), F32),
            pltpu.VMEM((S, 128), F32),
            pltpu.VMEM((S, D), A_x.dtype),
            pltpu.VMEM((3, D, HB, DHB), BF16),
            pltpu.VMEM((3, -(-(HB // 2) * (D + 1) // 8) * 8, DHB), U32),
            pltpu.VMEM((HB * DHB, D), BF16),
            pltpu.VMEM((HB * DHB // 2, D), U32),
            pltpu.SemaphoreType.DMA((NQ + 8,)),
            pltpu.SemaphoreType.DMA((NQ,)),
        ] + [pltpu.VMEM((BK, BQ), F32) for _ in range(2 * (S // BK))],
        compiler_params=pltpu.CompilerParams(vmem_limit_bytes=110 * 2**20),
    )(
        A_x.reshape(S, D), A_wqkv, A_wo, B_mem0.reshape(M, D), gate_w,
        B_Wq, B_Wk, B_Wv, B_Wo.reshape(HB * DHB, D),
    )
    return out.reshape(Bn, S, D)
```
